```python
import jax
import jax.numpy as jnp

def _softmax(x, axis=-1):
    return jax.nn.softmax(x, axis=axis)
def _gelu(x):
    return jax.nn.gelu(x, approximate=True)
def _silu(x):
    return jax.nn.silu(x)
def _sigmoid(x):
    return jax.nn.sigmoid(x)
def _layernorm(x, axis=-1, eps=1e-5):
    m = jnp.mean(x, axis=axis, keepdims=True)
    v = jnp.var(x, axis=axis, keepdims=True)
    return (x - m) / jnp.sqrt(v + eps)
def _scatter_add(tgt, idx, src, axis=0):
    return tgt.at[idx].add(src)
def _segment_sum(src, seg, n):
    return jax.ops.segment_sum(src, seg, n)
class _Rng:
    def __init__(self, key):
        self._k = key
    def _next(self):
        self._k, sub = jax.random.split(self._k)
        return sub
    def normal(self, shape):
        return jax.random.normal(self._next(), shape, dtype=jnp.bfloat16)
    def randint(self, lo, hi, shape):
        return jax.random.randint(self._next(), shape, lo, hi, dtype=jnp.int32)
    def uniform(self, shape, lo=0.0, hi=1.0):
        return jax.random.uniform(self._next(), shape, jnp.bfloat16, lo, hi)
    def permutation(self, n):
        return jax.random.permutation(self._next(), n)


kernel_name = 'standalone__structured_sparse_n_m__ragged'

def setup_inputs():
    _rng = _Rng(jax.random.key(int.from_bytes(__import__("os").urandom(4), "little")))
    _w = (lambda a: (lambda t: t.astype(jnp.bfloat16) if jnp.issubdtype(t.dtype, jnp.floating) else t)(jnp.asarray(a)))
    B, S, D = 16, 4096, 576
    assert D % 4 == 0, "d_model must be divisible by M=4 for 2:4 sparsity"
    return {
        "x": _w((lambda *s: _rng.normal(s) * 0.05)(B, S, D)),
        "w": _w((lambda *s: _rng.normal(s) * 0.05)(D, D)),
        "b": _w((lambda *s: _rng.normal(s) * 0.05)(D)),
    }

def reference(x, w, b):
    B, S, D = x.shape
    N, M = 2, 4
    G = D // M
    wg = w.reshape(G, M, D)
    mag = jnp.abs(wg)
    order = jnp.argsort(mag, 1)
    thr = jnp.take_along_axis(mag, order[:, M - N:M - N + 1, :], 1)
    mask = (lambda x, dt: x.astype(dt))(mag >= thr, w.dtype)
    wp = (wg * mask).reshape(D, D)
    return jnp.einsum("bsd,df->bsf", x, wp) + b
```

```python
import functools

import jax
import jax.numpy as jnp
import jax.experimental.pallas as pl
import jax.experimental.pallas.tpu as pltpu


def _prune_transpose(w_ref, wpt_ref, wf_ref):
    D = w_ref.shape[0]
    G = D // 4
    for c in range(pl.cdiv(D, 128)):
        lo = c * 128
        wd = min(128, D - lo)
        blk = w_ref[:, lo:lo + wd].astype(jnp.float32)
        if wd < 128:
            blk = jnp.concatenate([blk, jnp.zeros((D, 128 - wd), jnp.float32)], axis=1)
        wf_ref[...] = blk
        ws = [wf_ref[pl.ds(i, G, stride=4), :] for i in range(4)]
        ms = [jnp.abs(v) for v in ws]
        hi01 = jnp.maximum(ms[0], ms[1])
        lo01 = jnp.minimum(ms[0], ms[1])
        hi23 = jnp.maximum(ms[2], ms[3])
        lo23 = jnp.minimum(ms[2], ms[3])
        thr = jnp.maximum(jnp.minimum(hi01, hi23), jnp.maximum(lo01, lo23))
        for i in range(4):
            mask = (ms[i] >= thr).astype(jnp.float32)
            wf_ref[pl.ds(i, G, stride=4), :] = ws[i] * mask
        t = wf_ref[...].T
        wpt_ref[lo:lo + wd, :] = t[:wd, :].astype(jnp.bfloat16)


def _kernel(xt_ref, w_ref, b_ref, o_ref, wpt_ref, bcol_ref, wf_ref):
    D = w_ref.shape[0]

    @pl.when(jnp.logical_and(pl.program_id(0) == 0, pl.program_id(1) == 0))
    def _prep():
        _prune_transpose(w_ref, wpt_ref, wf_ref)
        brow = jnp.broadcast_to(b_ref[...].astype(jnp.float32), (128, D))
        bcol_ref[...] = brow.T

    acc = jnp.dot(wpt_ref[...], xt_ref[...], preferred_element_type=jnp.float32)
    ts = acc.shape[1]
    bias = jnp.tile(bcol_ref[...], (1, ts // 128))
    o_ref[...] = (acc + bias).astype(o_ref.dtype)


@functools.partial(jax.jit, static_argnames=("ts",))
def pallas_standalone__structured_sparse_n_m__ragged_kernel(
    x: jax.Array,
    w: jax.Array,
    b: jax.Array,
    ts: int = 2048,
):
    B, S, D = x.shape
    xt = jnp.swapaxes(x, 1, 2)
    b2 = b.reshape(1, D)
    out_t = pl.pallas_call(
        _kernel,
        grid=(B, S // ts),
        in_specs=[
            pl.BlockSpec((None, D, ts), lambda i, j: (i, 0, j)),
            pl.BlockSpec((D, D), lambda i, j: (0, 0)),
            pl.BlockSpec((1, D), lambda i, j: (0, 0)),
        ],
        out_specs=pl.BlockSpec((None, D, ts), lambda i, j: (i, 0, j)),
        out_shape=jax.ShapeDtypeStruct((B, D, S), x.dtype),
        scratch_shapes=[
            pltpu.VMEM((D, D), jnp.bfloat16),
            pltpu.VMEM((D, 128), jnp.float32),
            pltpu.VMEM((D, 128), jnp.float32),
        ],
        compiler_params=pltpu.CompilerParams(
            dimension_semantics=("arbitrary", "arbitrary"),
            vmem_limit_bytes=96 * 1024 * 1024,
        ),
    )(xt, w, b2)
    return jnp.swapaxes(out_t, 1, 2)
```

```python
import functools

import jax
import jax.numpy as jnp
from jax import lax
import jax.experimental.pallas as pl
import jax.experimental.pallas.tpu as pltpu

F32 = jnp.float32
BF16 = jnp.bfloat16

L_I, L_2, L_3, L_4, L_5, L_22, L_11 = 0, 2, 4, 6, 8, 10, 12
L_J, L_21, L_12 = 14, 15, 16
L_TMP = 17
NL = 19

RAMP = (256, 512, 1024, 2304)
BLOCKS = (512,) * 7 + (256, 256)
NSLOT = 3
OSUB = 128
NTAIL = 3
RC = 32


def _dot(a, b):
    return jnp.dot(a, b, preferred_element_type=F32)


def _mxu_transpose(v):
    r = lax.broadcasted_iota(jnp.int32, (128, 128), 0)
    c = lax.broadcasted_iota(jnp.int32, (128, 128), 1)
    eye = (r == c).astype(BF16)
    return lax.dot_general(eye, v, (((1,), (1,)), ((), ())), preferred_element_type=F32)


def _prune_rows(w_ref, pk_ref, at_ref, t):
    D = w_ref.shape[0]
    r0 = 128 * t
    nr = min(128, D - r0)
    G = nr // 4
    nc = pl.cdiv(D, 128)
    as_f32 = lambda v: lax.bitcast_convert_type(v, F32)
    mag, lo16, hi16 = 0x7FFF0000, 0x0000FFFF, -0x10000
    mx = None
    for c in range(nc):
        lo = c * 128
        wd = min(128, D - lo)
        u = pltpu.bitcast(w_ref[r0:r0 + nr, lo:lo + wd], jnp.int32)
        if wd < 128:
            u = jnp.concatenate([u, jnp.zeros((nr // 2, 128 - wd), jnp.int32)], axis=1)
        pk = pk_ref.at[t * nc + c]
        pk[0:nr // 2, :] = u
        a = pk[pl.ds(0, G, stride=2), :]
        b = pk[pl.ds(1, G, stride=2), :]
        e0 = as_f32((a << 16) & mag)
        e1 = as_f32(a & mag)
        e2 = as_f32((b << 16) & mag)
        e3 = as_f32(b & mag)
        thr = jnp.maximum(jnp.minimum(jnp.maximum(e0, e1), jnp.maximum(e2, e3)),
                          jnp.maximum(jnp.minimum(e0, e1), jnp.minimum(e2, e3)))
        pk[pl.ds(0, G, stride=2), :] = a & (jnp.where(e0 < thr, 0, lo16) | jnp.where(e1 < thr, 0, hi16))
        pk[pl.ds(1, G, stride=2), :] = b & (jnp.where(e2 < thr, 0, lo16) | jnp.where(e3 < thr, 0, hi16))
        u = pk[0:nr // 2, :]
        if nr < 128:
            u = jnp.concatenate([u, jnp.zeros((64 - nr // 2, 128), jnp.int32)], axis=0)
        p = pltpu.bitcast(u, BF16)
        if c < 2 and nr == 128:
            pf = _mxu_transpose(p)
            pt = pf.astype(BF16)
        else:
            pt = p.T
            pf = pt.astype(F32)
        at_ref[t, lo:lo + wd, :] = pt[:wd, :]
        m = jnp.max(jnp.abs(pf[:wd, :]).reshape(wd // 8, 8, 128), axis=0)
        mx = m if mx is None else jnp.maximum(mx, m)
    return jnp.max(mx, axis=0, keepdims=True)


def _pow2(m):
    e = jnp.minimum(lax.bitcast_convert_type(m, jnp.int32) & 0x7F800000, 253 << 23)
    return lax.bitcast_convert_type(e, F32), lax.bitcast_convert_type((254 << 23) - e, F32)


def _kernel(xt_hbm, w_hbm, b_hbm, o_hbm,
            xbuf, obuf, w_vmem, b_vmem, pk_ref, at_ref, drow_ref, dcol_ref, l_ref, bcol_ref, sems):
    B, D, S = xt_hbm.shape
    H = D // 2
    NP = S // OSUB
    HEADC = (NP - NTAIL) * OSUB
    SEM_W, SEM_B = 0, 3
    SEM_IN = 4
    SEM_HEAD = SEM_IN + NSLOT
    SEM_TAIL = SEM_HEAD + NSLOT
    SEM_RAMP = SEM_TAIL + NSLOT

    def in_copy(g, slot):
        return pltpu.make_async_copy(xt_hbm.at[g], xbuf.at[slot], sems.at[SEM_IN + slot])

    def start_out(g, slot, p0, p1):
        for p in range(p0, p1):
            c = p * OSUB
            sem = (SEM_HEAD if c < HEADC else SEM_TAIL) + slot
            pltpu.make_async_copy(obuf.at[slot, :, c:c + OSUB],
                                  o_hbm.at[g, :, c:c + OSUB], sems.at[sem]).start()

    def wait_head(slot):
        v = obuf.at[slot, :, 0:HEADC]
        pltpu.make_async_copy(v, v, sems.at[SEM_HEAD + slot]).wait()

    def wait_tail(slot):
        v = obuf.at[slot, :, HEADC:S]
        pltpu.make_async_copy(v, v, sems.at[SEM_TAIL + slot]).wait()

    def block(slot, c0, hh, msplit=1, direct_first=False):
        c1 = c0 + hh
        x = xbuf.at[slot]
        x1 = [x[64 * i:64 * (i + 1), c0:c0 + hh] for i in range(9)]
        x2 = [x[64 * i:64 * (i + 1), c1:c1 + hh] for i in range(9)]
        ds = [jnp.tile(dcol_ref[64 * i:64 * (i + 1), :], (1, hh // 128)) for i in range(8)]
        f1 = [v.astype(F32) * d for v, d in zip(x1, ds)]
        f2 = [v.astype(F32) * d for v, d in zip(x2, ds)]
        cat = lambda *vs: jnp.concatenate(vs, axis=0)
        add = lambda a, b: (a + b).astype(BF16)
        sub = lambda a, b: (a - b).astype(BF16)
        p = [add(f1[i], f2[i]) for i in range(8)]
        r_2 = cat(x1[0], x1[1], x1[4], x2[5])
        r_5 = cat(x2[2], x2[3], x2[6], x1[7])
        r_4 = cat(sub(f1[2], f1[0]), sub(f1[3], f1[1]), sub(f1[6], f1[4]), sub(f1[7], f1[5]))
        r_3 = cat(sub(f2[0], f2[2]), sub(f2[1], f2[3]), sub(f2[4], f2[6]), sub(f2[5], f2[7]))
        r_i = cat(add(f1[0], f2[2]), add(f1[1], f2[3]), add(f1[4], f2[6]))
        r_j = add(f2[5], f1[7])
        r_22 = cat(p[0], p[1], p[4], x2[8])
        r_11 = cat(p[2], p[3], p[6], x1[8])
        r_21 = cat(x1[8], p[5])
        r_12 = cat(x2[8], p[7])
        o = obuf.at[slot]
        mr = H // msplit
        for r0 in range(0, H, mr):
            def mm(i, r):
                k = r.shape[0]
                if k <= 128:
                    return _dot(l_ref[i, r0:r0 + mr, 0:k], r)
                lhs = jnp.concatenate(
                    [l_ref[i, r0:r0 + mr, :], l_ref[i + 1, r0:r0 + mr, 0:k - 128]], axis=1)
                return _dot(lhs, r)

            bias1 = jnp.tile(bcol_ref[r0:r0 + mr, :], (1, hh // 128))
            bias2 = jnp.tile(bcol_ref[H + r0:H + r0 + mr, :], (1, hh // 128))
            m2 = mm(L_2, r_2)
            if direct_first:
                m5 = mm(L_5, r_5)
            m4 = mm(L_4, r_4)
            if direct_first:
                m3 = mm(L_3, r_3)
            mj = mm(L_J, r_j)
            c21 = m2 + m4 + mj + mm(L_21, r_21) + bias2
            if not direct_first:
                m5 = mm(L_5, r_5)
                m3 = mm(L_3, r_3)
            c12 = m3 + m5 + mj + mm(L_12, r_12) + bias1
            mi = mm(L_I, r_i)
            c11 = (m4 - m5) + mi + mm(L_11, r_11) + bias1
            c22 = (m3 - m2) + mi + mm(L_22, r_22) + bias2
            o[H + r0:H + r0 + mr, c0:c0 + hh] = c21.astype(BF16)
            o[r0:r0 + mr, c1:c1 + hh] = c12.astype(BF16)
            o[r0:r0 + mr, c0:c0 + hh] = c11.astype(BF16)
            o[H + r0:H + r0 + mr, c1:c1 + hh] = c22.astype(BF16)

    w_cps = [pltpu.make_async_copy(w_hbm.at[a:b], w_vmem.at[a:b], sems.at[SEM_W + i])
             for i, (a, b) in enumerate([(0, 256), (256, 512), (512, D)])]
    b_cp = pltpu.make_async_copy(b_hbm, b_vmem, sems.at[SEM_B])
    offs = [sum(RAMP[:i]) for i in range(len(RAMP))]
    ramp_cps = [
        pltpu.make_async_copy(xt_hbm.at[0, :, o:o + sz], xbuf.at[0, :, o:o + sz], sems.at[SEM_RAMP + k])
        for k, (o, sz) in enumerate(zip(offs, RAMP))
    ]
    for cp in w_cps + [b_cp] + ramp_cps + [in_copy(1, 1), in_copy(2, 2)]:
        cp.start()

    low = lax.broadcasted_iota(jnp.int32, (RC, 128), 1) < 64
    low1 = lax.broadcasted_iota(jnp.int32, (1, 128), 1) < 64

    def prune_scaled(t):
        d, dinv = _pow2(_prune_rows(w_vmem, pk_ref, at_ref, t))
        drow_ref[t:t + 1, :] = d
        return d, dinv

    def make_dcol(t):
        dm = jnp.broadcast_to(drow_ref[t:t + 1, :], (128, 128)).astype(BF16)
        dcol_ref[128 * t:128 * (t + 1), :] = dm.T.astype(F32)

    def halves(t, r):
        return at_ref[t, r:r + RC, :].astype(F32), at_ref[t, H + r:H + r + RC, :].astype(F32)

    def put(i, r, v):
        l_ref[i, r:r + RC, :] = v.astype(BF16)

    w_cps[0].wait()
    d0, d0i = prune_scaled(0)
    d1, d1i = prune_scaled(1)
    for r in range(0, H, RC):
        p0, q0 = (v * d0i for v in halves(0, r))
        p1, q1 = (v * d1i for v in halves(1, r))
        put(L_2, r, (q0 + q1) * d0)
        put(L_5, r, (p0 + p1) * d1)
        put(L_4, r, q1)
        put(L_3, r, p0)
        put(L_I, r, p0 + q1)
        put(L_22, r, q0 - p0)
        put(L_11, r, p1 - q1)

    w_cps[1].wait()
    make_dcol(0)
    make_dcol(1)
    d2, d2i = prune_scaled(2)
    d3, d3i = prune_scaled(3)
    d2s = jnp.where(low1, d2, -d2)
    d3s = jnp.where(low1, d3, -d3)
    for r in range(0, H, RC):
        p2, q2 = (v * d2i for v in halves(2, r))
        p3, q3 = (v * d3i for v in halves(3, r))
        put(L_2 + 1, r, (q2 + q3) * d2s)
        put(L_5 + 1, r, (p2 + p3) * d3s)
        put(L_4 + 1, r, jnp.where(low, q3, -p2))
        put(L_3 + 1, r, jnp.where(low, p2, -q3))
        ij = p2 + q3
        put(L_I + 1, r, ij)
        put(L_J, r, pltpu.roll(ij, 64, 1))
        put(L_TMP, r, q2 - p2)
        put(L_TMP + 1, r, p3 - q3)

    w_cps[2].wait()
    b_cp.wait()
    ramp_cps[0].wait()
    make_dcol(2)
    make_dcol(3)
    _prune_rows(w_vmem, pk_ref, at_ref, 4)
    for r in range(0, H, RC):
        p4, q4 = halves(4, r)
        d21 = l_ref[L_TMP, r:r + RC, :].astype(F32)
        d12 = l_ref[L_TMP + 1, r:r + RC, :].astype(F32)
        put(L_21, r, jnp.where(low, q4, d21))
        put(L_12, r, jnp.where(low, p4, d12))
        put(L_22 + 1, r, jnp.where(low, d21, pltpu.roll(q4, 64, 1)))
        put(L_11 + 1, r, jnp.where(low, d12, pltpu.roll(p4, 64, 1)))
    brow = jnp.broadcast_to(b_vmem[...].astype(F32).reshape(1, D), (128, D))
    bcol_ref[...] = brow.astype(BF16).T.astype(F32)

    for k, (o, sz) in enumerate(zip(offs, RAMP)):
        if k > 0:
            ramp_cps[k].wait()
        c0, rem = o, sz
        while rem % 1024:
            hh, ms = (128, 3) if rem % 512 else (256, 2)
            block(0, c0, hh, msplit=ms, direct_first=(c0 == 0))
            c0 += 2 * hh
            rem -= 2 * hh
        for c in range(c0, o + sz, 512):
            block(0, c, 256)

    HP = NP // 2

    def body(g, slot):
        odd = g % 2 == 1
        even = jnp.logical_not(odd)
        last = g == B - 1
        nxt = jnp.where(slot == NSLOT - 1, 0, slot + 1)
        prv = jnp.where(slot == 0, NSLOT - 1, slot - 1)

        in_copy(g, slot).wait()
        pl.when(jnp.logical_and(even, g >= 4))(lambda: wait_head(slot))
        pl.when(g >= 3)(lambda: wait_tail(slot))
        pl.when(even)(lambda: wait_head(nxt))
        pl.when(even)(lambda: in_copy(g + 1, nxt).start())
        pl.when(jnp.logical_and(even, g + 2 < B))(lambda: in_copy(g + 2, prv).start())

        g_a = jnp.where(last, g - 1, g - 2)
        s_a = jnp.where(last, prv, nxt)
        prev_lo = lambda: start_out(g - 1, prv, 0, HP)
        prev_hi = lambda: start_out(g - 1, prv, HP, NP)
        odd_not_last = jnp.logical_and(odd, jnp.logical_not(last))
        after = {
            0: (jnp.logical_and(odd, g >= 3), lambda: start_out(g_a, s_a, HP, NP)),
            1: (odd_not_last, prev_lo),
            2: (odd_not_last, prev_hi),
            3: (g == B - 2, prev_lo),
            4: (g == B - 2, prev_hi),
            7: (jnp.logical_and(even, g < B - 2), prev_lo),
        }
        pl.when(last)(prev_lo)
        c = 0
        for j, bw in enumerate(BLOCKS):
            block(slot, c, bw // 2)
            if j in after:
                pl.when(after[j][0])(after[j][1])
            pl.when(last)(functools.partial(start_out, g, slot, c // OSUB, (c + bw) // OSUB))
            c += bw
        return nxt

    lax.fori_loop(1, B, body, 1)
    for s in range(NSLOT):
        wait_head(s)
        wait_tail(s)


@jax.jit
def pallas_standalone__structured_sparse_n_m__ragged_kernel(
    x: jax.Array,
    w: jax.Array,
    b: jax.Array,
):
    B, S, D = x.shape
    assert D == 576 and S == sum(RAMP) == sum(BLOCKS) and B % 2 == 0 and B >= 4
    nt = pl.cdiv(D, 128)
    out_t = pl.pallas_call(
        _kernel,
        in_specs=[pl.BlockSpec(memory_space=pl.ANY)] * 3,
        out_specs=pl.BlockSpec(memory_space=pl.ANY),
        out_shape=jax.ShapeDtypeStruct((B, D, S), x.dtype),
        scratch_shapes=[
            pltpu.VMEM((NSLOT, D, S), BF16),
            pltpu.VMEM((NSLOT, D, S), BF16),
            pltpu.VMEM((D, D), BF16),
            pltpu.VMEM((D,), BF16),
            pltpu.VMEM((nt * nt, 64, 128), jnp.int32),
            pltpu.VMEM((nt, D, 128), BF16),
            pltpu.VMEM((8, 128), F32),
            pltpu.VMEM((512, 128), F32),
            pltpu.VMEM((NL, D // 2, 128), BF16),
            pltpu.VMEM((D, 128), F32),
            pltpu.SemaphoreType.DMA((4 + 3 * NSLOT + len(RAMP),)),
        ],
        compiler_params=pltpu.CompilerParams(
            vmem_limit_bytes=64 * 1024 * 1024,
            disable_bounds_checks=True,
        ),
    )(jnp.swapaxes(x, 1, 2), w, b)
    return jnp.swapaxes(out_t, 1, 2)
```

```python
import functools

import jax
import jax.numpy as jnp
from jax import lax
import jax.experimental.pallas as pl
import jax.experimental.pallas.tpu as pltpu

F32 = jnp.float32
BF16 = jnp.bfloat16

L_I, L_2, L_3, L_4, L_5, L_22, L_11 = 0, 2, 4, 6, 8, 10, 12
L_J, L_21, L_12 = 14, 15, 16
L_TMP = 17
NL = 19

RAMP = (256, 512, 1024, 2304)
BLOCKS = (512,) * 7 + (256, 256)
NSLOT = 3
OSUB = 128
NTAIL = 3
RC = 32


def _dot(a, b):
    return jnp.dot(a, b, preferred_element_type=F32)


def _mxu_transpose(v):
    r = lax.broadcasted_iota(jnp.int32, (128, 128), 0)
    c = lax.broadcasted_iota(jnp.int32, (128, 128), 1)
    eye = (r == c).astype(BF16)
    return lax.dot_general(eye, v, (((1,), (1,)), ((), ())), preferred_element_type=F32)


def _prune_rows(w_ref, pk_ref, at_ref, t):
    D = w_ref.shape[0]
    r0 = 128 * t
    nr = min(128, D - r0)
    G = nr // 4
    nc = pl.cdiv(D, 128)
    as_f32 = lambda v: lax.bitcast_convert_type(v, F32)
    mag, lo16, hi16 = 0x7FFF0000, 0x0000FFFF, -0x10000
    mx = None
    for c in range(nc):
        lo = c * 128
        wd = min(128, D - lo)
        u = pltpu.bitcast(w_ref[r0:r0 + nr, lo:lo + wd], jnp.int32)
        if wd < 128:
            u = jnp.concatenate([u, jnp.zeros((nr // 2, 128 - wd), jnp.int32)], axis=1)
        pk = pk_ref.at[t * nc + c]
        pk[0:nr // 2, :] = u
        a = pk[pl.ds(0, G, stride=2), :]
        b = pk[pl.ds(1, G, stride=2), :]
        e0 = as_f32((a << 16) & mag)
        e1 = as_f32(a & mag)
        e2 = as_f32((b << 16) & mag)
        e3 = as_f32(b & mag)
        thr = jnp.maximum(jnp.minimum(jnp.maximum(e0, e1), jnp.maximum(e2, e3)),
                          jnp.maximum(jnp.minimum(e0, e1), jnp.minimum(e2, e3)))
        pk[pl.ds(0, G, stride=2), :] = a & (jnp.where(e0 < thr, 0, lo16) | jnp.where(e1 < thr, 0, hi16))
        pk[pl.ds(1, G, stride=2), :] = b & (jnp.where(e2 < thr, 0, lo16) | jnp.where(e3 < thr, 0, hi16))
        u = pk[0:nr // 2, :]
        if nr < 128:
            u = jnp.concatenate([u, jnp.zeros((64 - nr // 2, 128), jnp.int32)], axis=0)
        p = pltpu.bitcast(u, BF16)
        if c < 2 and nr == 128:
            pf = _mxu_transpose(p)
            pt = pf.astype(BF16)
        else:
            pt = p.T
            pf = pt.astype(F32)
        at_ref[t, lo:lo + wd, :] = pt[:wd, :]
        m = jnp.max(jnp.abs(pf[:wd, :]).reshape(wd // 8, 8, 128), axis=0)
        mx = m if mx is None else jnp.maximum(mx, m)
    return jnp.max(mx, axis=0, keepdims=True)


def _pow2(m):
    e = jnp.minimum(lax.bitcast_convert_type(m, jnp.int32) & 0x7F800000, 253 << 23)
    return lax.bitcast_convert_type(e, F32), lax.bitcast_convert_type((254 << 23) - e, F32)


def _kernel(xt_hbm, w_hbm, b_hbm, o_hbm,
            xbuf, obuf, w_vmem, b_vmem, pk_ref, at_ref, drow_ref, dcol_ref, l_ref, bcol_ref, sems):
    B, D, S = xt_hbm.shape
    H = D // 2
    NP = S // OSUB
    HEADC = (NP - NTAIL) * OSUB
    SEM_W, SEM_B = 0, 3
    SEM_IN = 4
    SEM_HEAD = SEM_IN + NSLOT
    SEM_TAIL = SEM_HEAD + NSLOT
    SEM_RAMP = SEM_TAIL + NSLOT

    def in_copy(g, slot):
        return pltpu.make_async_copy(xt_hbm.at[g], xbuf.at[slot], sems.at[SEM_IN + slot])

    def start_out(g, slot, p0, p1):
        for p in range(p0, p1):
            c = p * OSUB
            sem = (SEM_HEAD if c < HEADC else SEM_TAIL) + slot
            pltpu.make_async_copy(obuf.at[slot, :, c:c + OSUB],
                                  o_hbm.at[g, :, c:c + OSUB], sems.at[sem]).start()

    def wait_head(slot):
        v = obuf.at[slot, :, 0:HEADC]
        pltpu.make_async_copy(v, v, sems.at[SEM_HEAD + slot]).wait()

    def wait_tail(slot):
        v = obuf.at[slot, :, HEADC:S]
        pltpu.make_async_copy(v, v, sems.at[SEM_TAIL + slot]).wait()

    def block(slot, c0, hh, msplit=1, direct_first=False):
        c1 = c0 + hh
        x = xbuf.at[slot]
        x1 = [x[64 * i:64 * (i + 1), c0:c0 + hh] for i in range(9)]
        x2 = [x[64 * i:64 * (i + 1), c1:c1 + hh] for i in range(9)]
        ds = [jnp.tile(dcol_ref[64 * i:64 * (i + 1), :], (1, hh // 128)) for i in range(8)]
        f1 = [v.astype(F32) * d for v, d in zip(x1, ds)]
        f2 = [v.astype(F32) * d for v, d in zip(x2, ds)]
        cat = lambda *vs: jnp.concatenate(vs, axis=0)
        add = lambda a, b: (a + b).astype(BF16)
        sub = lambda a, b: (a - b).astype(BF16)
        p = [add(f1[i], f2[i]) for i in range(8)]
        r_2 = cat(x1[0], x1[1], x1[4], x2[5])
        r_5 = cat(x2[2], x2[3], x2[6], x1[7])
        r_4 = cat(sub(f1[2], f1[0]), sub(f1[3], f1[1]), sub(f1[6], f1[4]), sub(f1[7], f1[5]))
        r_3 = cat(sub(f2[0], f2[2]), sub(f2[1], f2[3]), sub(f2[4], f2[6]), sub(f2[5], f2[7]))
        r_i = cat(add(f1[0], f2[2]), add(f1[1], f2[3]), add(f1[4], f2[6]))
        r_j = add(f2[5], f1[7])
        r_22 = cat(p[0], p[1], p[4], x2[8])
        r_11 = cat(p[2], p[3], p[6], x1[8])
        r_21 = cat(x1[8], p[5])
        r_12 = cat(x2[8], p[7])
        o = obuf.at[slot]
        mr = H // msplit
        for r0 in range(0, H, mr):
            def mm(i, r):
                k = r.shape[0]
                if k <= 128:
                    return _dot(l_ref[i, r0:r0 + mr, 0:k], r)
                lhs = jnp.concatenate(
                    [l_ref[i, r0:r0 + mr, :], l_ref[i + 1, r0:r0 + mr, 0:k - 128]], axis=1)
                return _dot(lhs, r)

            bias1 = jnp.tile(bcol_ref[r0:r0 + mr, :], (1, hh // 128))
            bias2 = jnp.tile(bcol_ref[H + r0:H + r0 + mr, :], (1, hh // 128))
            m2 = mm(L_2, r_2)
            if direct_first:
                m5 = mm(L_5, r_5)
            m4 = mm(L_4, r_4)
            if direct_first:
                m3 = mm(L_3, r_3)
            mj = mm(L_J, r_j)
            c21 = m2 + m4 + mj + mm(L_21, r_21) + bias2
            if not direct_first:
                m5 = mm(L_5, r_5)
                m3 = mm(L_3, r_3)
            c12 = m3 + m5 + mj + mm(L_12, r_12) + bias1
            mi = mm(L_I, r_i)
            c11 = (m4 - m5) + mi + mm(L_11, r_11) + bias1
            c22 = (m3 - m2) + mi + mm(L_22, r_22) + bias2
            o[H + r0:H + r0 + mr, c0:c0 + hh] = c21.astype(BF16)
            o[r0:r0 + mr, c1:c1 + hh] = c12.astype(BF16)
            o[r0:r0 + mr, c0:c0 + hh] = c11.astype(BF16)
            o[H + r0:H + r0 + mr, c1:c1 + hh] = c22.astype(BF16)

    w_cps = [pltpu.make_async_copy(w_hbm.at[a:b], w_vmem.at[a:b], sems.at[SEM_W + i])
             for i, (a, b) in enumerate([(0, 256), (256, 512), (512, D)])]
    b_cp = pltpu.make_async_copy(b_hbm, b_vmem, sems.at[SEM_B])
    offs = [sum(RAMP[:i]) for i in range(len(RAMP))]
    ramp_cps = [
        pltpu.make_async_copy(xt_hbm.at[0, :, o:o + sz], xbuf.at[0, :, o:o + sz], sems.at[SEM_RAMP + k])
        for k, (o, sz) in enumerate(zip(offs, RAMP))
    ]
    for cp in w_cps + [b_cp] + ramp_cps + [in_copy(1, 1), in_copy(2, 2)]:
        cp.start()

    low = lax.broadcasted_iota(jnp.int32, (RC, 128), 1) < 64
    low1 = lax.broadcasted_iota(jnp.int32, (1, 128), 1) < 64

    def prune_scaled(t):
        d, dinv = _pow2(_prune_rows(w_vmem, pk_ref, at_ref, t))
        drow_ref[t:t + 1, :] = d
        return d, dinv

    def make_dcol(t):
        dm = jnp.broadcast_to(drow_ref[t:t + 1, :], (128, 128)).astype(BF16)
        dcol_ref[128 * t:128 * (t + 1), :] = dm.T.astype(F32)

    def halves(t, r):
        return at_ref[t, r:r + RC, :].astype(F32), at_ref[t, H + r:H + r + RC, :].astype(F32)

    def put(i, r, v):
        l_ref[i, r:r + RC, :] = v.astype(BF16)

    w_cps[0].wait()
    d0, d0i = prune_scaled(0)
    d1, d1i = prune_scaled(1)
    for r in range(0, H, RC):
        p0, q0 = (v * d0i for v in halves(0, r))
        p1, q1 = (v * d1i for v in halves(1, r))
        put(L_2, r, (q0 + q1) * d0)
        put(L_5, r, (p0 + p1) * d1)
        put(L_4, r, q1)
        put(L_3, r, p0)
        put(L_I, r, p0 + q1)
        put(L_22, r, q0 - p0)
        put(L_11, r, p1 - q1)

    w_cps[1].wait()
    make_dcol(0)
    make_dcol(1)
    d2, d2i = prune_scaled(2)
    d3, d3i = prune_scaled(3)
    d2s = jnp.where(low1, d2, -d2)
    d3s = jnp.where(low1, d3, -d3)
    for r in range(0, H, RC):
        p2, q2 = (v * d2i for v in halves(2, r))
        p3, q3 = (v * d3i for v in halves(3, r))
        put(L_2 + 1, r, (q2 + q3) * d2s)
        put(L_5 + 1, r, (p2 + p3) * d3s)
        put(L_4 + 1, r, jnp.where(low, q3, -p2))
        put(L_3 + 1, r, jnp.where(low, p2, -q3))
        ij = p2 + q3
        put(L_I + 1, r, ij)
        put(L_J, r, pltpu.roll(ij, 64, 1))
        put(L_TMP, r, q2 - p2)
        put(L_TMP + 1, r, p3 - q3)

    w_cps[2].wait()
    b_cp.wait()
    ramp_cps[0].wait()
    make_dcol(2)
    make_dcol(3)
    _prune_rows(w_vmem, pk_ref, at_ref, 4)
    for r in range(0, H, RC):
        p4, q4 = halves(4, r)
        d21 = l_ref[L_TMP, r:r + RC, :].astype(F32)
        d12 = l_ref[L_TMP + 1, r:r + RC, :].astype(F32)
        put(L_21, r, jnp.where(low, q4, d21))
        put(L_12, r, jnp.where(low, p4, d12))
        put(L_22 + 1, r, jnp.where(low, d21, pltpu.roll(q4, 64, 1)))
        put(L_11 + 1, r, jnp.where(low, d12, pltpu.roll(p4, 64, 1)))
    brow = jnp.broadcast_to(b_vmem[...].astype(F32).reshape(1, D), (128, D))
    bcol_ref[...] = brow.astype(BF16).T.astype(F32)

    for k, (o, sz) in enumerate(zip(offs, RAMP)):
        if k > 0:
            ramp_cps[k].wait()
        c0, rem = o, sz
        while rem % 1024:
            hh, ms = (128, 3) if rem % 512 else (256, 2)
            block(0, c0, hh, msplit=ms, direct_first=(c0 == 0))
            c0 += 2 * hh
            rem -= 2 * hh
        for c in range(c0, o + sz, 512):
            block(0, c, 256)

    HP = NP // 2

    def body(g, state):
        slot, nxt, prv, parity = state
        odd = parity == 1
        even = jnp.logical_not(odd)
        last = g == B - 1

        in_copy(g, slot).wait()
        pl.when(jnp.logical_and(even, g >= 4))(lambda: wait_head(slot))
        pl.when(g >= 3)(lambda: wait_tail(slot))
        pl.when(even)(lambda: wait_head(nxt))
        pl.when(even)(lambda: in_copy(g + 1, nxt).start())
        pl.when(jnp.logical_and(even, g + 2 < B))(lambda: in_copy(g + 2, prv).start())

        g_a = jnp.where(last, g - 1, g - 2)
        s_a = jnp.where(last, prv, nxt)
        prev_lo = lambda: start_out(g - 1, prv, 0, HP)
        prev_hi = lambda: start_out(g - 1, prv, HP, NP)
        odd_not_last = jnp.logical_and(odd, jnp.logical_not(last))
        after = {
            0: (jnp.logical_and(odd, g >= 3), lambda: start_out(g_a, s_a, HP, NP)),
            1: (odd_not_last, prev_lo),
            2: (odd_not_last, prev_hi),
            3: (g == B - 2, prev_lo),
            4: (g == B - 2, prev_hi),
            7: (jnp.logical_and(even, g < B - 2), prev_lo),
        }
        pl.when(last)(prev_lo)
        c = 0
        for j, bw in enumerate(BLOCKS):
            block(slot, c, bw // 2)
            if j in after:
                pl.when(after[j][0])(after[j][1])
            pl.when(last)(functools.partial(start_out, g, slot, c // OSUB, (c + bw) // OSUB))
            c += bw
        return nxt, prv, slot, 1 - parity

    lax.fori_loop(1, B, body, (1, 2, 0, 1))
    for s in range(NSLOT):
        wait_head(s)
        wait_tail(s)


@jax.jit
def pallas_standalone__structured_sparse_n_m__ragged_kernel(
    x: jax.Array,
    w: jax.Array,
    b: jax.Array,
):
    B, S, D = x.shape
    assert D == 576 and S == sum(RAMP) == sum(BLOCKS) and B % 2 == 0 and B >= 4
    nt = pl.cdiv(D, 128)
    out_t = pl.pallas_call(
        _kernel,
        in_specs=[pl.BlockSpec(memory_space=pl.ANY)] * 3,
        out_specs=pl.BlockSpec(memory_space=pl.ANY),
        out_shape=jax.ShapeDtypeStruct((B, D, S), x.dtype),
        scratch_shapes=[
            pltpu.VMEM((NSLOT, D, S), BF16),
            pltpu.VMEM((NSLOT, D, S), BF16),
            pltpu.VMEM((D, D), BF16),
            pltpu.VMEM((D,), BF16),
            pltpu.VMEM((nt * nt, 64, 128), jnp.int32),
            pltpu.VMEM((nt, D, 128), BF16),
            pltpu.VMEM((8, 128), F32),
            pltpu.VMEM((512, 128), F32),
            pltpu.VMEM((NL, D // 2, 128), BF16),
            pltpu.VMEM((D, 128), F32),
            pltpu.SemaphoreType.DMA((4 + 3 * NSLOT + len(RAMP),)),
        ],
        compiler_params=pltpu.CompilerParams(
            vmem_limit_bytes=64 * 1024 * 1024,
            disable_bounds_checks=True,
            disable_semaphore_checks=True,
        ),
    )(jnp.swapaxes(x, 1, 2), w, b)
    return jnp.swapaxes(out_t, 1, 2)
```

```python
import functools

import jax
import jax.numpy as jnp
from jax import lax
import jax.experimental.pallas as pl
import jax.experimental.pallas.tpu as pltpu

F32 = jnp.float32
BF16 = jnp.bfloat16

L_I, L_2, L_3, L_4, L_5, L_22, L_11 = 0, 2, 4, 6, 8, 10, 12
L_J, L_21, L_12 = 14, 15, 16
L_TMP = 17
NL = 19

RAMP = (256, 512, 1280)
MID = 2048
BLOCKS = (512,) * 7 + (256, 256)
OSUB = 128
NTAIL = 8
LAG = 2048
WSTART = 7
W0_AFTER = 1
RC = 32


def _dot(a, b):
    return jnp.dot(a, b, preferred_element_type=F32)


def _mxu_transpose(v):
    r = lax.broadcasted_iota(jnp.int32, (128, 128), 0)
    c = lax.broadcasted_iota(jnp.int32, (128, 128), 1)
    eye = (r == c).astype(BF16)
    return lax.dot_general(eye, v, (((1,), (1,)), ((), ())), preferred_element_type=F32)


def _prune_rows(w_ref, pk_ref, at_ref, t):
    D = w_ref.shape[0]
    r0 = 128 * t
    nr = min(128, D - r0)
    G = nr // 4
    nc = pl.cdiv(D, 128)
    as_f32 = lambda v: lax.bitcast_convert_type(v, F32)
    mag, lo16, hi16 = 0x7FFF0000, 0x0000FFFF, -0x10000
    mx = None
    for c in range(nc):
        lo = c * 128
        wd = min(128, D - lo)
        u = pltpu.bitcast(w_ref[r0:r0 + nr, lo:lo + wd], jnp.int32)
        if wd < 128:
            u = jnp.concatenate([u, jnp.zeros((nr // 2, 128 - wd), jnp.int32)], axis=1)
        pk = pk_ref.at[t * nc + c]
        pk[0:nr // 2, :] = u
        a = pk[pl.ds(0, G, stride=2), :]
        b = pk[pl.ds(1, G, stride=2), :]
        e0 = as_f32((a << 16) & mag)
        e1 = as_f32(a & mag)
        e2 = as_f32((b << 16) & mag)
        e3 = as_f32(b & mag)
        thr = jnp.maximum(jnp.minimum(jnp.maximum(e0, e1), jnp.maximum(e2, e3)),
                          jnp.maximum(jnp.minimum(e0, e1), jnp.minimum(e2, e3)))
        pk[pl.ds(0, G, stride=2), :] = a & (jnp.where(e0 < thr, 0, lo16) | jnp.where(e1 < thr, 0, hi16))
        pk[pl.ds(1, G, stride=2), :] = b & (jnp.where(e2 < thr, 0, lo16) | jnp.where(e3 < thr, 0, hi16))
        u = pk[0:nr // 2, :]
        if nr < 128:
            u = jnp.concatenate([u, jnp.zeros((64 - nr // 2, 128), jnp.int32)], axis=0)
        p = pltpu.bitcast(u, BF16)
        if c < 2 and nr == 128:
            pf = _mxu_transpose(p)
            pt = pf.astype(BF16)
        else:
            pt = p.T
            pf = pt.astype(F32)
        at_ref[t, lo:lo + wd, :] = pt[:wd, :]
        m = jnp.max(jnp.abs(pf[:wd, :]).reshape(wd // 8, 8, 128), axis=0)
        mx = m if mx is None else jnp.maximum(mx, m)
    return jnp.max(mx, axis=0, keepdims=True)


def _pow2(m):
    e = jnp.minimum(lax.bitcast_convert_type(m, jnp.int32) & 0x7F800000, 253 << 23)
    return lax.bitcast_convert_type(e, F32), lax.bitcast_convert_type((254 << 23) - e, F32)


def _kernel(xt_hbm, w_hbm, b_hbm, o_hbm,
            xbuf, obuf, w_vmem, b_vmem, pk_ref, at_ref, drow_ref, dcol_ref, l_ref, bcol_ref, sems):
    B, D, S = xt_hbm.shape
    H = D // 2
    NPAIR = B // 2
    NMID = (2 * S - sum(RAMP)) // MID
    SEM_W, SEM_B = 0, 3
    SEM_IN = 4
    SEM_HEAD = 6
    SEM_TAIL = 7
    SEM_MISC = 9
    SEM_RAMP = 10
    SEM_MID = SEM_RAMP + len(RAMP)

    def in_pair(p, half):
        return pltpu.make_async_copy(xt_hbm.at[pl.ds(2 * p, 2)], xbuf.at[pl.ds(2 * half, 2)],
                                     sems.at[SEM_IN + half])

    def out_piece(g, buf, c, sem):
        pltpu.make_async_copy(obuf.at[buf, :, c:c + OSUB], o_hbm.at[g, :, c:c + OSUB], sems.at[sem]).start()

    def wait_cols(n, sem):
        assert n % (2 * OSUB) == 0
        v = obuf.at[0:2, :, 0:n // 2]
        pltpu.make_async_copy(v, v, sems.at[sem]).wait()

    def block(x, o, c0, hh, msplit=1, direct_first=False):
        c1 = c0 + hh
        x1 = [x[64 * i:64 * (i + 1), c0:c0 + hh] for i in range(9)]
        x2 = [x[64 * i:64 * (i + 1), c1:c1 + hh] for i in range(9)]
        ds = [jnp.tile(dcol_ref[64 * i:64 * (i + 1), :], (1, hh // 128)) for i in range(8)]
        f1 = [v.astype(F32) * d for v, d in zip(x1, ds)]
        f2 = [v.astype(F32) * d for v, d in zip(x2, ds)]
        cat = lambda *vs: jnp.concatenate(vs, axis=0)
        add = lambda a, b: (a + b).astype(BF16)
        sub = lambda a, b: (a - b).astype(BF16)
        p = [add(f1[i], f2[i]) for i in range(8)]
        r_2 = cat(x1[0], x1[1], x1[4], x2[5])
        r_5 = cat(x2[2], x2[3], x2[6], x1[7])
        r_4 = cat(sub(f1[2], f1[0]), sub(f1[3], f1[1]), sub(f1[6], f1[4]), sub(f1[7], f1[5]))
        r_3 = cat(sub(f2[0], f2[2]), sub(f2[1], f2[3]), sub(f2[4], f2[6]), sub(f2[5], f2[7]))
        r_i = cat(add(f1[0], f2[2]), add(f1[1], f2[3]), add(f1[4], f2[6]))
        r_j = add(f2[5], f1[7])
        r_22 = cat(p[0], p[1], p[4], x2[8])
        r_11 = cat(p[2], p[3], p[6], x1[8])
        r_21 = cat(x1[8], p[5])
        r_12 = cat(x2[8], p[7])
        mr = H // msplit
        for r0 in range(0, H, mr):
            def mm(i, r):
                k = r.shape[0]
                if k <= 128:
                    return _dot(l_ref[i, r0:r0 + mr, 0:k], r)
                lhs = jnp.concatenate(
                    [l_ref[i, r0:r0 + mr, :], l_ref[i + 1, r0:r0 + mr, 0:k - 128]], axis=1)
                return _dot(lhs, r)

            bias1 = jnp.tile(bcol_ref[r0:r0 + mr, :], (1, hh // 128))
            bias2 = jnp.tile(bcol_ref[H + r0:H + r0 + mr, :], (1, hh // 128))
            m2 = mm(L_2, r_2)
            if direct_first:
                m5 = mm(L_5, r_5)
            m4 = mm(L_4, r_4)
            if direct_first:
                m3 = mm(L_3, r_3)
            mj = mm(L_J, r_j)
            c21 = m2 + m4 + mj + mm(L_21, r_21) + bias2
            if not direct_first:
                m5 = mm(L_5, r_5)
                m3 = mm(L_3, r_3)
            c12 = m3 + m5 + mj + mm(L_12, r_12) + bias1
            mi = mm(L_I, r_i)
            c11 = (m4 - m5) + mi + mm(L_11, r_11) + bias1
            c22 = (m3 - m2) + mi + mm(L_22, r_22) + bias2
            o[H + r0:H + r0 + mr, c0:c0 + hh] = c21.astype(BF16)
            o[r0:r0 + mr, c1:c1 + hh] = c12.astype(BF16)
            o[r0:r0 + mr, c0:c0 + hh] = c11.astype(BF16)
            o[H + r0:H + r0 + mr, c1:c1 + hh] = c22.astype(BF16)

    w_cps = [pltpu.make_async_copy(w_hbm.at[a:b], w_vmem.at[a:b], sems.at[SEM_W + i])
             for i, (a, b) in enumerate([(0, 256), (256, 512), (512, D)])]
    b_cp = pltpu.make_async_copy(b_hbm, b_vmem, sems.at[SEM_B])
    offs = [sum(RAMP[:i]) for i in range(len(RAMP))]
    ramp_cps = [
        pltpu.make_async_copy(xt_hbm.at[0, :, o:o + sz], xbuf.at[0, :, o:o + sz], sems.at[SEM_RAMP + k])
        for k, (o, sz) in enumerate(zip(offs, RAMP))
    ]

    def mid_copy(k):
        u = k + 1
        g, c = u // (S // MID), (u % (S // MID)) * MID
        if not isinstance(k, int):
            c = pl.multiple_of(c, MID)
        return pltpu.make_async_copy(xt_hbm.at[g, :, pl.ds(c, MID)], xbuf.at[g, :, pl.ds(c, MID)],
                                     sems.at[SEM_MID + k]), g, c

    for cp in w_cps + [b_cp] + ramp_cps + [mid_copy(k)[0] for k in range(NMID)] + [in_pair(1, 1)]:
        cp.start()

    low = lax.broadcasted_iota(jnp.int32, (RC, 128), 1) < 64
    low1 = lax.broadcasted_iota(jnp.int32, (1, 128), 1) < 64

    def prune_scaled(t):
        d, dinv = _pow2(_prune_rows(w_vmem, pk_ref, at_ref, t))
        drow_ref[t:t + 1, :] = d
        return d, dinv

    def make_dcol(t):
        dm = jnp.broadcast_to(drow_ref[t:t + 1, :], (128, 128)).astype(BF16)
        dcol_ref[128 * t:128 * (t + 1), :] = dm.T.astype(F32)

    def halves(t, r):
        return at_ref[t, r:r + RC, :].astype(F32), at_ref[t, H + r:H + r + RC, :].astype(F32)

    def put(i, r, v):
        l_ref[i, r:r + RC, :] = v.astype(BF16)

    w_cps[0].wait()
    d0, d0i = prune_scaled(0)
    d1, d1i = prune_scaled(1)
    for r in range(0, H, RC):
        p0, q0 = (v * d0i for v in halves(0, r))
        p1, q1 = (v * d1i for v in halves(1, r))
        put(L_2, r, (q0 + q1) * d0)
        put(L_5, r, (p0 + p1) * d1)
        put(L_4, r, q1)
        put(L_3, r, p0)
        put(L_I, r, p0 + q1)
        put(L_22, r, q0 - p0)
        put(L_11, r, p1 - q1)

    w_cps[1].wait()
    make_dcol(0)
    make_dcol(1)
    d2, d2i = prune_scaled(2)
    d3, d3i = prune_scaled(3)
    make_dcol(2)
    make_dcol(3)
    d2s = jnp.where(low1, d2, -d2)
    d3s = jnp.where(low1, d3, -d3)
    for r in range(0, H, RC):
        p2, q2 = (v * d2i for v in halves(2, r))
        p3, q3 = (v * d3i for v in halves(3, r))
        put(L_2 + 1, r, (q2 + q3) * d2s)
        put(L_5 + 1, r, (p2 + p3) * d3s)
        put(L_4 + 1, r, jnp.where(low, q3, -p2))
        put(L_3 + 1, r, jnp.where(low, p2, -q3))
        ij = p2 + q3
        put(L_I + 1, r, ij)
        put(L_J, r, pltpu.roll(ij, 64, 1))
        put(L_TMP, r, q2 - p2)
        put(L_TMP + 1, r, p3 - q3)

    w_cps[2].wait()
    b_cp.wait()
    ramp_cps[0].wait()
    _prune_rows(w_vmem, pk_ref, at_ref, 4)
    for r in range(0, H, RC):
        p4, q4 = halves(4, r)
        d21 = l_ref[L_TMP, r:r + RC, :].astype(F32)
        d12 = l_ref[L_TMP + 1, r:r + RC, :].astype(F32)
        put(L_21, r, jnp.where(low, q4, d21))
        put(L_12, r, jnp.where(low, p4, d12))
        put(L_22 + 1, r, jnp.where(low, d21, pltpu.roll(q4, 64, 1)))
        put(L_11 + 1, r, jnp.where(low, d12, pltpu.roll(p4, 64, 1)))
    brow = jnp.broadcast_to(b_vmem[...].astype(F32).reshape(1, D), (128, D))
    bcol_ref[...] = brow.astype(BF16).T.astype(F32)

    for k, (o, sz) in enumerate(zip(offs, RAMP)):
        if k > 0:
            ramp_cps[k].wait()
        c0, rem = o, sz
        while rem % 1024:
            hh, ms = (128, 3) if rem % 512 else (256, 2)
            block(xbuf.at[0], obuf.at[0], c0, hh, msplit=ms, direct_first=(c0 == 0))
            c0 += 2 * hh
            rem -= 2 * hh
        for c in range(c0, o + sz, 512):
            block(xbuf.at[0], obuf.at[0], c, 256)

    def mid_body(k, carry):
        cp, g, c = mid_copy(k)
        cp.wait()
        x = xbuf.at[g, :, pl.ds(c, MID)]
        o = obuf.at[g, :, pl.ds(c, MID)]
        for j in range(MID // 512):
            block(x, o, 512 * j, 256)
            if j == W0_AFTER:
                @pl.when(k == NMID - 1)
                def _():
                    for cc in range(0, LAG, OSUB):
                        out_piece(0, 0, cc, SEM_MISC)
        return carry

    lax.fori_loop(0, NMID, mid_body, 0)

    NWIN = 2 * S // OSUB

    def body(p, half):
        other = 1 - half
        last = p == NPAIR - 1
        not_last = jnp.logical_not(last)
        in_pair(p, half).wait()
        pl.when(p >= 2)(lambda: wait_cols((NWIN - NTAIL) * OSUB, SEM_HEAD))
        pl.when(p >= 3)(lambda: wait_cols(NTAIL * OSUB, SEM_TAIL + half))
        pl.when(p == 2)(lambda: wait_cols(LAG, SEM_MISC))
        pl.when(not_last)(lambda: in_pair(p + 1, other).start())

        def window(i0, i1):
            for i in range(i0, i1):
                db, c = divmod(LAG + i * OSUB, S)
                buf = 2 * half if db == 2 else 2 * other + db
                out_piece(2 * p - 2 + db, buf, c, SEM_TAIL + half if i >= NWIN - NTAIL else SEM_HEAD)

        nprev = (2 * S - LAG) // OSUB
        early = [(lo, min(lo + 12, nprev)) for lo in range(0, nprev, 12)]
        pl.when(last)(functools.partial(window, *early[0]))
        j = 0
        for i in range(2):
            c = 0
            for bw in BLOCKS:
                block(xbuf.at[2 * half + i], obuf.at[2 * half + i], c, bw // 2)
                if 0 <= j - WSTART < NWIN // 16:
                    pl.when(not_last)(functools.partial(window, 16 * (j - WSTART), 16 * (j - WSTART + 1)))
                if j + 1 < len(early):
                    pl.when(last)(functools.partial(window, *early[j + 1]))

                @pl.when(last)
                def _():
                    for cc in range(c, c + bw, OSUB):
                        if i == 0 and cc < LAG:
                            window(nprev + cc // OSUB, nprev + cc // OSUB + 1)
                        else:
                            out_piece(2 * p + i, 2 * half + i, cc, SEM_MISC)
                c += bw
                j += 1
        return other

    lax.fori_loop(1, NPAIR, body, 1)
    wait_cols((NWIN - NTAIL) * OSUB, SEM_HEAD)
    wait_cols(NTAIL * OSUB, SEM_TAIL)
    wait_cols(NTAIL * OSUB, SEM_TAIL + 1)
    wait_cols(2 * S - LAG, SEM_MISC)


@jax.jit
def pallas_standalone__structured_sparse_n_m__ragged_kernel(
    x: jax.Array,
    w: jax.Array,
    b: jax.Array,
):
    B, S, D = x.shape
    assert D == 576 and S == sum(BLOCKS) and sum(RAMP) == MID and S % MID == 0 and B % 2 == 0 and B >= 6
    assert NTAIL * OSUB <= LAG <= MID
    nt = pl.cdiv(D, 128)
    out_t = pl.pallas_call(
        _kernel,
        in_specs=[pl.BlockSpec(memory_space=pl.ANY)] * 3,
        out_specs=pl.BlockSpec(memory_space=pl.ANY),
        out_shape=jax.ShapeDtypeStruct((B, D, S), x.dtype),
        scratch_shapes=[
            pltpu.VMEM((4, D, S), BF16),
            pltpu.VMEM((4, D, S), BF16),
            pltpu.VMEM((D, D), BF16),
            pltpu.VMEM((D,), BF16),
            pltpu.VMEM((nt * nt, 64, 128), jnp.int32),
            pltpu.VMEM((nt, D, 128), BF16),
            pltpu.VMEM((8, 128), F32),
            pltpu.VMEM((512, 128), F32),
            pltpu.VMEM((NL, D // 2, 128), BF16),
            pltpu.VMEM((D, 128), F32),
            pltpu.SemaphoreType.DMA((10 + len(RAMP) + 3,)),
        ],
        compiler_params=pltpu.CompilerParams(
            vmem_limit_bytes=64 * 1024 * 1024,
            disable_bounds_checks=True,
            disable_semaphore_checks=True,
        ),
    )(jnp.swapaxes(x, 1, 2), w, b)
    return jnp.swapaxes(out_t, 1, 2)
```

```python
import functools
from fractions import Fraction

import jax
import jax.numpy as jnp
from jax import lax
import jax.experimental.pallas as pl
import jax.experimental.pallas.tpu as pltpu

F32 = jnp.float32
BF16 = jnp.bfloat16

PAIRS = ((0, 2), (1, 3), (4, 6), (5, 7), (8, None))
_H, _Q, _T = Fraction(1, 2), Fraction(1, 4), Fraction(1, 3)
PASSES = (
    ((0, (1, 0, 0, 1), (1, 0, -1, -1)), (4, (_T, 0, _T, 0), (1, -1, 0, 0)), (1, -1, 0, -1)),
    ((0, (0, 0, 1, 1), (1, 0, 0, 0)), (3, (0, 1, 0, 1), (0, 0, 1, -1)), (0, 0, 1, 0)),
    ((0, (1, 0, 0, 0), (1, 1, -1, -1)), (2, (-_H, 0, -_H, 0), (1, -1, 0, 0)), (0, 1, 0, 1)),
    ((0, (0, 0, 0, -1), (1, 0, -1, 0)), (3, (_Q, 0, _Q, 0), (1, -1, 0, 0)), (1, -1, 1, -1)),
    ((0, (1, 1, 0, 0), (0, 0, 1, 1)), (2, (0, 1, 0, 1), (0, 0, 1, -1)), (1, 0, 0, 0)),
    ((0, (-1, 0, 1, 0), (0, 1, 0, 0)), (1, (-1, 0, -1, 0), (1, -1, 0, 0)), (0, 0, 0, 1)),
    ((0, (0, -1, 0, 1), (0, 0, 0, 1)), (1, (0, _H, 0, _H), (0, 0, 1, -1)), (1, -1, 0, 0)),
    ((4, (-_T, 0, _T, 0), (0, 1, 0, 0)), (1, (_H, 0, 0, -_H), (2, 0, -1, -1)), (1, -1, 0, 2)),
    ((1, (0, 0, 1, 1), (1, 0, 0, 0)), (3, (-1, -1, 1, 1), (0, 0, 0, 1)), (0, 0, 1, 1)),
    ((2, (_H, 0, -_H, 0), (0, 1, 0, -1)), (1, (1, 0, 0, 0), (1, 1, -1, -1)), (0, 1, 0, -1)),
    ((1, (0, 0, 0, 1), (1, 0, -1, 0)), (3, (-_H, 0, _H, 0), (0, 1, 0, -1)), (1, -1, -1, 1)),
    ((2, (1, 1, -1, -1), (0, 0, 0, 1)), (1, (_H, _H, 0, 0), (0, 0, 1, 1)), (1, 1, 0, 0)),
    ((2, (_H, 0, -_H, -1), (1, 0, 0, -1)), (4, (_T, 0, 0, 0), (1, 1, 0, 0)), (2, 1, 0, 1)),
    ((2, (0, 0, 1, 1), (1, 0, 0, 0)), (3, (_H, _H, 0, 0), (1, 1, 0, 0)), (1, 1, 1, 1)),
    ((2, (0, 0, 0, 1), (1, 0, -1, 0)), (3, (0, -1, 0, 0), (1, 1, -1, -1)), (1, 0, -1, 0)),
    ((4, (0, 0, -_T, 0), (1, 0, 0, 0)), (3, (_Q, _H, -_Q, 0), (1, 1, 0, -2)), (1, -1, -3, -1)),
)


def _check_scheme():
    for pair, (_, kb) in enumerate(PAIRS):
        members = 1 if kb is None else 2
        for ia in range(4):
            for ix in range(4):
                for ic in range(4):
                    got = sum(ac[ia] * xc[ix] * out[ic]
                              for *slots, out in PASSES for p, ac, xc in slots if p == pair)
                    want = (ia % 2 == ix // 2 < members and ic == 2 * (ia // 2) + ix % 2)
                    assert got == int(want)


_X_RECIPE = {
    (1, 1, 0, 0): ((1, 0, 0, 0), 1, (0, 1, 0, 0)),
    (1, -1, 0, 0): ((1, 0, 0, 0), -1, (0, 1, 0, 0)),
    (0, 0, 1, 1): ((0, 0, 1, 0), 1, (0, 0, 0, 1)),
    (0, 0, 1, -1): ((0, 0, 1, 0), -1, (0, 0, 0, 1)),
    (1, 0, -1, 0): ((1, 0, 0, 0), -1, (0, 0, 1, 0)),
    (0, 1, 0, -1): ((0, 1, 0, 0), -1, (0, 0, 0, 1)),
    (1, 0, 0, -1): ((1, 0, 0, 0), -1, (0, 0, 0, 1)),
    (1, 0, -1, -1): ((1, 0, 0, 0), -1, (0, 0, 1, 1)),
    (1, 1, -1, -1): ((1, 1, 0, 0), -1, (0, 0, 1, 1)),
    (2, 0, -1, -1): ((1, 1, -1, -1), 1, (1, -1, 0, 0)),
    (1, 1, 0, -2): ((1, 0, 0, -1), 1, (0, 1, 0, -1)),
}
_X_RECIPE_PAIR3 = {**_X_RECIPE, (1, 1, -1, -1): ((1, 1, 0, -2), -1, (0, 0, 1, -1))}

RAMP = (256, 512, 1024, 2304)
BW = 256
OSUB = 128
WTAIL = 2
RTAIL = 64
PRE = 8
WRITE_EARLY = (13, 13)
READ_EARLY = (14,)
RC = 16


def _dot(a, b):
    return jnp.dot(a, b, preferred_element_type=F32)


def _mxu_transpose(v):
    r = lax.broadcasted_iota(jnp.int32, (128, 128), 0)
    c = lax.broadcasted_iota(jnp.int32, (128, 128), 1)
    eye = (r == c).astype(BF16)
    return lax.dot_general(eye, v, (((1,), (1,)), ((), ())), preferred_element_type=F32)


def _prune_rows(w_ref, pk_ref, at_ref, t):
    D = w_ref.shape[0]
    r0 = 128 * t
    nr = min(128, D - r0)
    G = nr // 4
    nc = pl.cdiv(D, 128)
    as_f32 = lambda v: lax.bitcast_convert_type(v, F32)
    mag, lo16, hi16 = 0x7FFF0000, 0x0000FFFF, -0x10000
    mx = None
    for c in range(nc):
        lo = c * 128
        wd = min(128, D - lo)
        u = pltpu.bitcast(w_ref[r0:r0 + nr, lo:lo + wd], jnp.int32)
        if wd < 128:
            u = jnp.concatenate([u, jnp.zeros((nr // 2, 128 - wd), jnp.int32)], axis=1)
        pk = pk_ref.at[t * nc + c]
        pk[0:nr // 2, :] = u
        a = pk[pl.ds(0, G, stride=2), :]
        b = pk[pl.ds(1, G, stride=2), :]
        e0 = as_f32((a << 16) & mag)
        e1 = as_f32(a & mag)
        e2 = as_f32((b << 16) & mag)
        e3 = as_f32(b & mag)
        thr = jnp.maximum(jnp.minimum(jnp.maximum(e0, e1), jnp.maximum(e2, e3)),
                          jnp.maximum(jnp.minimum(e0, e1), jnp.minimum(e2, e3)))
        pk[pl.ds(0, G, stride=2), :] = a & (jnp.where(e0 < thr, 0, lo16) | jnp.where(e1 < thr, 0, hi16))
        pk[pl.ds(1, G, stride=2), :] = b & (jnp.where(e2 < thr, 0, lo16) | jnp.where(e3 < thr, 0, hi16))
        u = pk[0:nr // 2, :]
        if nr < 128:
            u = jnp.concatenate([u, jnp.zeros((64 - nr // 2, 128), jnp.int32)], axis=0)
        p = pltpu.bitcast(u, BF16)
        if c < 2 and nr == 128:
            pf = _mxu_transpose(p)
            pt = pf.astype(BF16)
        else:
            pt = p.T
            pf = pt.astype(F32)
        at_ref[t, lo:lo + wd, :] = pt[:wd, :]
        m = jnp.max(jnp.abs(pf[:wd, :]).reshape(wd // 8, 8, 128), axis=0)
        mx = m if mx is None else jnp.maximum(mx, m)
    return jnp.max(mx, axis=0, keepdims=True)


def _pow2(m):
    e = jnp.minimum(lax.bitcast_convert_type(m, jnp.int32) & 0x7F800000, 253 << 23)
    return lax.bitcast_convert_type(e, F32), lax.bitcast_convert_type((254 << 23) - e, F32)


def _is_plain(xc):
    return sum(abs(t) for t in xc) == 1


def _kernel(xt_hbm, w_hbm, b_hbm, o_hbm,
            xbuf, obuf, w_vmem, b_vmem, pk_ref, at_ref, drow_ref, dcol_ref, l_ref, bcol_ref, sems):
    B, D, S = xt_hbm.shape
    H = D // 2
    NP = S // OSUB
    SEM_W, SEM_B = 0, 3
    SEM_RMAIN, SEM_RTAIL = 4, 5
    SEM_WMAIN, SEM_WTAIL = 7, 8
    SEM_X1, SEM_LAST = 9, 10
    SEM_RAMP = 11

    def start_reads(g, buf):
        cut = D - RTAIL
        pltpu.make_async_copy(xt_hbm.at[g], xbuf.at[buf], sems.at[SEM_RMAIN]).start()
        pltpu.make_async_copy(xt_hbm.at[g + 1, 0:cut], xbuf.at[buf + 1, 0:cut], sems.at[SEM_RMAIN]).start()
        pltpu.make_async_copy(xt_hbm.at[g + 1, cut:D], xbuf.at[buf + 1, cut:D],
                              sems.at[SEM_RTAIL + (buf >> 1)]).start()

    def write(g, buf, p0, p1, sem, tail_sem=None, in_order=False):
        for p in range(p0, p1):
            c = (p if in_order else (2 * p if 2 * p < NP else 2 * p - NP + 1)) * OSUB
            s = tail_sem if tail_sem is not None and p >= NP - WTAIL else sem
            pltpu.make_async_copy(obuf.at[buf, :, c:c + OSUB], o_hbm.at[g, :, c:c + OSUB], sems.at[s]).start()

    def wait_all(sem, rows=None, cols=None):
        v = xbuf.at[0:2, 0:rows // 2] if cols is None else obuf.at[0:2, :, 0:cols // 2]
        pltpu.make_async_copy(v, v, sems.at[sem]).wait()

    def block(buf, c0):
        x, o = xbuf.at[buf], obuf.at[buf]
        cols = (c0, c0 + BW // 2)
        raw = lambda k, l: x[64 * k:64 * (k + 1), cols[l]:cols[l] + BW // 2]
        cache = {}

        def comb(pair, xc):
            if (pair, xc) not in cache:
                if _is_plain(xc):
                    i = xc.index(1)
                    k = PAIRS[pair][i // 2]
                    v = raw(k, i % 2).astype(F32)
                    if pair < 4:
                        v = v * dcol_ref[64 * k:64 * (k + 1), :]
                else:
                    u, sign, w = (_X_RECIPE_PAIR3 if pair == 3 else _X_RECIPE)[xc]
                    v = comb(pair, u) + comb(pair, w) if sign > 0 else comb(pair, u) - comb(pair, w)
                cache[pair, xc] = v
            return cache[pair, xc]

        def operand(pair, xc):
            if _is_plain(xc):
                i = xc.index(1)
                return raw(PAIRS[pair][i // 2], i % 2)
            return comb(pair, xc).astype(BF16)

        def mm(i):
            return _dot(l_ref[i], jnp.concatenate([operand(p, xc) for p, _, xc in PASSES[i][:2]], axis=0))

        def store(i, l, v):
            o[i * H:(i + 1) * H, cols[l]:cols[l] + BW // 2] = v.astype(BF16)

        bias1, bias2 = bcol_ref[0:H, :], bcol_ref[H:D, :]
        p0, p3, p10, p15 = mm(0), mm(3), mm(10), mm(15)
        v = p3 - p10
        e = p0 + p15
        g = e + (p3 + p10)
        c21 = bias2 + v - 3.0 * p15
        c22 = bias2 - v - e
        p6, p7, p2, p9 = mm(6), mm(7), mm(2), mm(9)
        g = g + p6 + p7
        c11 = bias1 + g
        c12 = bias1 - g + p2 + p9
        c22 = c22 + 2.0 * p7 + p2 - p9
        p11, p12, p13, p8 = mm(11), mm(12), mm(13), mm(8)
        h = p11 + p12 + p13
        u = p8 + p13
        c11 = c11 + h + p12
        store(0, 1, c12 + h)
        c21 = c21 + u
        c22 = c22 + u + p12
        p1, p4, p5, p14 = mm(1), mm(4), mm(5), mm(14)
        store(0, 0, c11 + p4 + p14)
        store(1, 0, c21 + p1 - p14)
        store(1, 1, c22 + p5)

    w_cps = [pltpu.make_async_copy(w_hbm.at[a:b], w_vmem.at[a:b], sems.at[SEM_W + i])
             for i, (a, b) in enumerate([(0, 256), (256, 512), (512, D)])]
    b_cp = pltpu.make_async_copy(b_hbm, b_vmem, sems.at[SEM_B])
    offs = [sum(RAMP[:i]) for i in range(len(RAMP))]
    ramp_cps = [
        pltpu.make_async_copy(xt_hbm.at[0, :, o:o + sz], xbuf.at[0, :, o:o + sz], sems.at[SEM_RAMP + k])
        for k, (o, sz) in enumerate(zip(offs, RAMP))
    ]
    x1_cp = pltpu.make_async_copy(xt_hbm.at[1], xbuf.at[1], sems.at[SEM_X1])
    for cp in w_cps + [b_cp] + ramp_cps + [x1_cp]:
        cp.start()
    start_reads(2, 2)

    def prune_scaled(t):
        d, dinv = _pow2(_prune_rows(w_vmem, pk_ref, at_ref, t))
        drow_ref[t:t + 1, :] = d
        return d, dinv

    def make_dcol(t):
        dm = jnp.broadcast_to(drow_ref[t:t + 1, :], (128, 128)).astype(BF16)
        dcol_ref[128 * t:128 * (t + 1), :] = dm.T.astype(F32)

    w_cps[0].wait()
    scale = [prune_scaled(0), prune_scaled(1)]
    w_cps[1].wait()
    make_dcol(0)
    make_dcol(1)
    scale += [prune_scaled(2), prune_scaled(3)]
    w_cps[2].wait()
    make_dcol(2)
    make_dcol(3)
    _prune_rows(w_vmem, pk_ref, at_ref, 4)
    low = lax.broadcasted_iota(jnp.int32, (RC, 128), 1) < 64
    for r in range(0, H, RC):
        a = {}
        for t in range(5):
            for i in range(2):
                v = at_ref[t, i * H + r:i * H + r + RC, :].astype(F32)
                a[i, t] = v * scale[t][1] if t < 4 else v

        def slot_value(pair, ac, xc, half):
            ks = PAIRS[pair]
            m = max(abs(t) for t in ac)
            v = None
            for j, t in enumerate(ac):
                if t != 0:
                    s = a[j // 2, ks[j % 2] // 2]
                    if abs(t) != m:
                        s = s * float(abs(t) / m)
                    v = (s if t > 0 else -s) if v is None else (v + s if t > 0 else v - s)
            if _is_plain(xc) and pair < 4:
                v = v * (scale[ks[xc.index(1) // 2] // 2][0] * float(m))
            elif m != 1:
                v = v * float(m)
            return v if ks[0] % 2 == half else pltpu.roll(v, 64, 1)

        for i, (s0, s1, _) in enumerate(PASSES):
            l_ref[i, r:r + RC, :] = jnp.where(low, slot_value(*s0, 0), slot_value(*s1, 1)).astype(BF16)
    b_cp.wait()
    ramp_cps[0].wait()
    brow = jnp.broadcast_to(b_vmem[...].astype(F32).reshape(1, D), (128, D))
    bcol_ref[...] = brow.astype(BF16).T.astype(F32)

    for k, (o, sz) in enumerate(zip(offs, RAMP)):
        if k > 0:
            ramp_cps[k].wait()
        for c in range(o, o + sz, BW):
            block(0, c)

    HP = NP // 2

    def body(g, buf):
        odd = (buf & 1) == 1
        even = jnp.logical_not(odd)
        last = g == B - 1
        inner_odd = jnp.logical_and(odd, jnp.logical_and(g > 1, jnp.logical_not(last)))
        buf2 = buf ^ 2
        buf1 = jnp.where(buf == 0, 3, buf - 1)

        pl.when(g == 1)(lambda: x1_cp.wait())
        pl.when(even)(lambda: wait_all(SEM_RMAIN, rows=2 * D - RTAIL))
        pl.when(jnp.logical_and(odd, g > 1))(lambda: wait_all(SEM_RTAIL + (buf >> 1), rows=RTAIL))
        pl.when(inner_odd)(lambda: wait_all(SEM_WMAIN, cols=2 * S - WTAIL * OSUB))
        pl.when(jnp.logical_and(even, g >= 4))(lambda: wait_all(SEM_WTAIL, cols=WTAIL * OSUB))

        pl.when(jnp.logical_and(inner_odd, g > 2 * len(READ_EARLY) + 1))(lambda: start_reads(g + 1, buf2 - 1))
        pl.when(jnp.logical_and(even, g > 2 * len(WRITE_EARLY)))(lambda: write(g - 2, buf2, 0, PRE, SEM_WMAIN))
        pl.when(even)(lambda: write(g - 2, buf2, PRE, HP, SEM_WMAIN))
        after = {
            0: [(even, lambda: write(g - 2, buf2, HP, NP, SEM_WMAIN)),
                (last, lambda: write(g - 1, buf1, 0, HP - 2, SEM_LAST))],
            1: [(even, lambda: write(g - 1, buf1, 0, HP, SEM_WMAIN)),
                (last, lambda: write(g - 1, buf1, HP - 2, NP - 4, SEM_LAST))],
            2: [(even, lambda: write(g - 1, buf1, HP, NP, SEM_WMAIN, SEM_WTAIL)),
                (last, lambda: write(g - 1, buf1, NP - 4, NP, SEM_LAST))],
        }
        for i, j in enumerate(WRITE_EARLY):
            after.setdefault(j, []).append(
                (g == 2 * i + 1, functools.partial(write, 2 * i, 2 * i % 4, 0, PRE, SEM_WMAIN)))
        for i, j in enumerate(READ_EARLY):
            after.setdefault(j, []).append(
                (g == 2 * i + 2, functools.partial(start_reads, 2 * i + 4, 2 * i % 4)))
        ppb = BW // OSUB
        for j in range(S // BW):
            block(buf, j * BW)
            for cond, fn in after.get(j, []):
                pl.when(cond)(fn)
            if j >= 2:
                pl.when(last)(functools.partial(write, g, buf, 0 if j == 2 else j * ppb, (j + 1) * ppb,
                                                SEM_LAST, in_order=True))
        return (buf + 1) & 3

    lax.fori_loop(1, B, body, 1)
    wait_all(SEM_WMAIN, cols=2 * S - WTAIL * OSUB)
    wait_all(SEM_WTAIL, cols=WTAIL * OSUB)
    wait_all(SEM_LAST, cols=2 * S)


@jax.jit
def pallas_standalone__structured_sparse_n_m__ragged_kernel(
    x: jax.Array,
    w: jax.Array,
    b: jax.Array,
):
    B, S, D = x.shape
    assert D == 576 and S == sum(RAMP) and BW == 256 and B % 2 == 0 and WTAIL % 2 == 0
    assert B >= 2 * max(len(WRITE_EARLY), len(READ_EARLY) + 1, 1) + 2
    _check_scheme()
    nt = pl.cdiv(D, 128)
    out_t = pl.pallas_call(
        _kernel,
        in_specs=[pl.BlockSpec(memory_space=pl.ANY)] * 3,
        out_specs=pl.BlockSpec(memory_space=pl.ANY),
        out_shape=jax.ShapeDtypeStruct((B, D, S), x.dtype),
        scratch_shapes=[
            pltpu.VMEM((4, D, S), BF16),
            pltpu.VMEM((4, D, S), BF16),
            pltpu.VMEM((D, D), BF16),
            pltpu.VMEM((D,), BF16),
            pltpu.VMEM((nt * nt, 64, 128), jnp.int32),
            pltpu.VMEM((nt, D, 128), BF16),
            pltpu.VMEM((8, 128), F32),
            pltpu.VMEM((512, 128), F32),
            pltpu.VMEM((len(PASSES), D // 2, 128), BF16),
            pltpu.VMEM((D, 128), F32),
            pltpu.SemaphoreType.DMA((11 + len(RAMP),)),
        ],
        compiler_params=pltpu.CompilerParams(
            vmem_limit_bytes=64 * 1024 * 1024,
            disable_bounds_checks=True,
            disable_semaphore_checks=True,
        ),
    )(jnp.swapaxes(x, 1, 2), w, b)
    return jnp.swapaxes(out_t, 1, 2)
```

```python
import functools
from fractions import Fraction

import jax
import jax.numpy as jnp
from jax import lax
import jax.experimental.pallas as pl
import jax.experimental.pallas.tpu as pltpu

F32 = jnp.float32
BF16 = jnp.bfloat16

PAIRS = ((0, 2), (1, 3), (4, 6), (5, 7), (8, None))
_H, _Q, _T = Fraction(1, 2), Fraction(1, 4), Fraction(1, 3)
PASSES = (
    ((0, (1, 0, 0, 1), (1, 0, -1, -1)), (4, (_T, 0, _T, 0), (1, -1, 0, 0)), (1, -1, 0, -1)),
    ((0, (0, 0, 1, 1), (1, 0, 0, 0)), (3, (0, 1, 0, 1), (0, 0, 1, -1)), (0, 0, 1, 0)),
    ((0, (1, 0, 0, 0), (1, 1, -1, -1)), (2, (-_H, 0, -_H, 0), (1, -1, 0, 0)), (0, 1, 0, 1)),
    ((0, (0, 0, 0, -1), (1, 0, -1, 0)), (3, (_Q, 0, _Q, 0), (1, -1, 0, 0)), (1, -1, 1, -1)),
    ((0, (1, 1, 0, 0), (0, 0, 1, 1)), (2, (0, 1, 0, 1), (0, 0, 1, -1)), (1, 0, 0, 0)),
    ((0, (-1, 0, 1, 0), (0, 1, 0, 0)), (1, (-1, 0, -1, 0), (1, -1, 0, 0)), (0, 0, 0, 1)),
    ((0, (0, -1, 0, 1), (0, 0, 0, 1)), (1, (0, _H, 0, _H), (0, 0, 1, -1)), (1, -1, 0, 0)),
    ((4, (-_T, 0, _T, 0), (0, 1, 0, 0)), (1, (_H, 0, 0, -_H), (2, 0, -1, -1)), (1, -1, 0, 2)),
    ((1, (0, 0, 1, 1), (1, 0, 0, 0)), (3, (-1, -1, 1, 1), (0, 0, 0, 1)), (0, 0, 1, 1)),
    ((2, (_H, 0, -_H, 0), (0, 1, 0, -1)), (1, (1, 0, 0, 0), (1, 1, -1, -1)), (0, 1, 0, -1)),
    ((1, (0, 0, 0, 1), (1, 0, -1, 0)), (3, (-_H, 0, _H, 0), (0, 1, 0, -1)), (1, -1, -1, 1)),
    ((2, (1, 1, -1, -1), (0, 0, 0, 1)), (1, (_H, _H, 0, 0), (0, 0, 1, 1)), (1, 1, 0, 0)),
    ((2, (_H, 0, -_H, -1), (1, 0, 0, -1)), (4, (_T, 0, 0, 0), (1, 1, 0, 0)), (2, 1, 0, 1)),
    ((2, (0, 0, 1, 1), (1, 0, 0, 0)), (3, (_H, _H, 0, 0), (1, 1, 0, 0)), (1, 1, 1, 1)),
    ((2, (0, 0, 0, 1), (1, 0, -1, 0)), (3, (0, -1, 0, 0), (1, 1, -1, -1)), (1, 0, -1, 0)),
    ((4, (0, 0, -_T, 0), (1, 0, 0, 0)), (3, (_Q, _H, -_Q, 0), (1, 1, 0, -2)), (1, -1, -3, -1)),
)


def _check_scheme():
    for pair, (_, kb) in enumerate(PAIRS):
        members = 1 if kb is None else 2
        for ia in range(4):
            for ix in range(4):
                for ic in range(4):
                    got = sum(ac[ia] * xc[ix] * out[ic]
                              for *slots, out in PASSES for p, ac, xc in slots if p == pair)
                    want = (ia % 2 == ix // 2 < members and ic == 2 * (ia // 2) + ix % 2)
                    assert got == int(want)


_X_RECIPE = {
    (1, 1, 0, 0): ((1, 0, 0, 0), 1, (0, 1, 0, 0)),
    (1, -1, 0, 0): ((1, 0, 0, 0), -1, (0, 1, 0, 0)),
    (0, 0, 1, 1): ((0, 0, 1, 0), 1, (0, 0, 0, 1)),
    (0, 0, 1, -1): ((0, 0, 1, 0), -1, (0, 0, 0, 1)),
    (1, 0, -1, 0): ((1, 0, 0, 0), -1, (0, 0, 1, 0)),
    (0, 1, 0, -1): ((0, 1, 0, 0), -1, (0, 0, 0, 1)),
    (1, 0, 0, -1): ((1, 0, 0, 0), -1, (0, 0, 0, 1)),
    (1, 0, -1, -1): ((1, 0, 0, 0), -1, (0, 0, 1, 1)),
    (1, 1, -1, -1): ((1, 1, 0, 0), -1, (0, 0, 1, 1)),
    (2, 0, -1, -1): ((1, 1, -1, -1), 1, (1, -1, 0, 0)),
    (1, 1, 0, -2): ((1, 0, 0, -1), 1, (0, 1, 0, -1)),
}
_X_RECIPE_PAIR3 = {**_X_RECIPE, (1, 1, -1, -1): ((1, 1, 0, -2), -1, (0, 0, 1, -1))}

RAMP = (256, 512, 1024, 2304)
BW = 256
OSUB = 128
WTAIL = 2
RTAIL = 64
PRE = 10
RC = 16


def _dot(a, b):
    return jnp.dot(a, b, preferred_element_type=F32)


def _mxu_transpose(v):
    r = lax.broadcasted_iota(jnp.int32, (128, 128), 0)
    c = lax.broadcasted_iota(jnp.int32, (128, 128), 1)
    eye = (r == c).astype(BF16)
    return lax.dot_general(eye, v, (((1,), (1,)), ((), ())), preferred_element_type=F32)


def _prune_rows(w_ref, pk_ref, at_ref, t):
    D = w_ref.shape[0]
    r0 = 128 * t
    nr = min(128, D - r0)
    G = nr // 4
    nc = pl.cdiv(D, 128)
    as_f32 = lambda v: lax.bitcast_convert_type(v, F32)
    mag, lo16, hi16 = 0x7FFF0000, 0x0000FFFF, -0x10000
    mx = None
    for c in range(nc):
        lo = c * 128
        wd = min(128, D - lo)
        u = pltpu.bitcast(w_ref[r0:r0 + nr, lo:lo + wd], jnp.int32)
        if wd < 128:
            u = jnp.concatenate([u, jnp.zeros((nr // 2, 128 - wd), jnp.int32)], axis=1)
        pk = pk_ref.at[t * nc + c]
        pk[0:nr // 2, :] = u
        a = pk[pl.ds(0, G, stride=2), :]
        b = pk[pl.ds(1, G, stride=2), :]
        e0 = as_f32((a << 16) & mag)
        e1 = as_f32(a & mag)
        e2 = as_f32((b << 16) & mag)
        e3 = as_f32(b & mag)
        thr = jnp.maximum(jnp.minimum(jnp.maximum(e0, e1), jnp.maximum(e2, e3)),
                          jnp.maximum(jnp.minimum(e0, e1), jnp.minimum(e2, e3)))
        pk[pl.ds(0, G, stride=2), :] = a & (jnp.where(e0 < thr, 0, lo16) | jnp.where(e1 < thr, 0, hi16))
        pk[pl.ds(1, G, stride=2), :] = b & (jnp.where(e2 < thr, 0, lo16) | jnp.where(e3 < thr, 0, hi16))
        u = pk[0:nr // 2, :]
        if nr < 128:
            u = jnp.concatenate([u, jnp.zeros((64 - nr // 2, 128), jnp.int32)], axis=0)
        p = pltpu.bitcast(u, BF16)
        if c < 2 and nr == 128:
            pf = _mxu_transpose(p)
            pt = pf.astype(BF16)
        else:
            pt = p.T
            pf = pt.astype(F32)
        at_ref[t, lo:lo + wd, :] = pt[:wd, :]
        m = jnp.max(jnp.abs(pf[:wd, :]).reshape(wd // 8, 8, 128), axis=0)
        mx = m if mx is None else jnp.maximum(mx, m)
    return jnp.max(mx, axis=0, keepdims=True)


def _pow2(m):
    e = jnp.minimum(lax.bitcast_convert_type(m, jnp.int32) & 0x7F800000, 253 << 23)
    return lax.bitcast_convert_type(e, F32), lax.bitcast_convert_type((254 << 23) - e, F32)


def _is_plain(xc):
    return sum(abs(t) for t in xc) == 1


def _kernel(xt_hbm, w_hbm, b_hbm, o_hbm,
            xbuf, obuf, w_vmem, b_vmem, pk_ref, at_ref, drow_ref, dcol_ref, l_ref, bcol_ref, sems):
    B, D, S = xt_hbm.shape
    H = D // 2
    NP = S // OSUB
    SEM_W, SEM_B = 0, 3
    SEM_RMAIN, SEM_RTAIL = 4, 5
    SEM_WMAIN, SEM_WTAIL = 6, 7
    SEM_X1, SEM_X23, SEM_LAST = 8, 9, 10
    SEM_RAMP = 11

    def start_reads(g, buf):
        cut = D - RTAIL
        pltpu.make_async_copy(xt_hbm.at[pl.ds(g, 3)], xbuf.at[pl.ds(buf, 3)], sems.at[SEM_RMAIN]).start()
        pltpu.make_async_copy(xt_hbm.at[g + 3, 0:cut], xbuf.at[buf + 3, 0:cut], sems.at[SEM_RMAIN]).start()
        pltpu.make_async_copy(xt_hbm.at[g + 3, cut:D], xbuf.at[buf + 3, cut:D], sems.at[SEM_RTAIL]).start()

    def write(g, buf, p0, p1, sem, tail_sem=None, in_order=False):
        for p in range(p0, p1):
            c = (p if in_order else (2 * p if 2 * p < NP else 2 * p - NP + 1)) * OSUB
            s = tail_sem if tail_sem is not None and p >= NP - WTAIL else sem
            pltpu.make_async_copy(obuf.at[buf, :, c:c + OSUB], o_hbm.at[g, :, c:c + OSUB], sems.at[s]).start()

    def wait_all(sem, rows=None, tiles=None):
        if tiles is None:
            v = xbuf.at[0:4, 0:rows // 4]
        else:
            n = min(k for k in range(1, 9) if tiles % k == 0 and tiles // k <= NP)
            v = obuf.at[0:n, :, 0:tiles // n * OSUB]
        pltpu.make_async_copy(v, v, sems.at[sem]).wait()

    def block(buf, c0):
        x, o = xbuf.at[buf], obuf.at[buf]
        cols = (c0, c0 + BW // 2)
        raw = lambda k, l: x[64 * k:64 * (k + 1), cols[l]:cols[l] + BW // 2]
        cache = {}

        def comb(pair, xc):
            if (pair, xc) not in cache:
                if _is_plain(xc):
                    i = xc.index(1)
                    k = PAIRS[pair][i // 2]
                    v = raw(k, i % 2).astype(F32)
                    if pair < 4:
                        v = v * dcol_ref[64 * k:64 * (k + 1), :]
                else:
                    u, sign, w = (_X_RECIPE_PAIR3 if pair == 3 else _X_RECIPE)[xc]
                    v = comb(pair, u) + comb(pair, w) if sign > 0 else comb(pair, u) - comb(pair, w)
                cache[pair, xc] = v
            return cache[pair, xc]

        def operand(pair, xc):
            if _is_plain(xc):
                i = xc.index(1)
                return raw(PAIRS[pair][i // 2], i % 2)
            return comb(pair, xc).astype(BF16)

        def mm(i):
            return _dot(l_ref[i], jnp.concatenate([operand(p, xc) for p, _, xc in PASSES[i][:2]], axis=0))

        def store(i, l, v):
            o[i * H:(i + 1) * H, cols[l]:cols[l] + BW // 2] = v.astype(BF16)

        bias1, bias2 = bcol_ref[0:H, :], bcol_ref[H:D, :]
        p0, p3, p10, p15 = mm(0), mm(3), mm(10), mm(15)
        v = p3 - p10
        e = p0 + p15
        g = e + (p3 + p10)
        c21 = bias2 + v - 3.0 * p15
        c22 = bias2 - v - e
        p6, p7, p2, p9 = mm(6), mm(7), mm(2), mm(9)
        g = g + p6 + p7
        c11 = bias1 + g
        c12 = bias1 - g + p2 + p9
        c22 = c22 + 2.0 * p7 + p2 - p9
        p11, p12, p13, p8 = mm(11), mm(12), mm(13), mm(8)
        h = p11 + p12 + p13
        u = p8 + p13
        c11 = c11 + h + p12
        store(0, 1, c12 + h)
        c21 = c21 + u
        c22 = c22 + u + p12
        p1, p4, p5, p14 = mm(1), mm(4), mm(5), mm(14)
        store(0, 0, c11 + p4 + p14)
        store(1, 0, c21 + p1 - p14)
        store(1, 1, c22 + p5)

    w_cps = [pltpu.make_async_copy(w_hbm.at[a:b], w_vmem.at[a:b], sems.at[SEM_W + i])
             for i, (a, b) in enumerate([(0, 256), (256, 512), (512, D)])]
    b_cp = pltpu.make_async_copy(b_hbm, b_vmem, sems.at[SEM_B])
    offs = [sum(RAMP[:i]) for i in range(len(RAMP))]
    ramp_cps = [
        pltpu.make_async_copy(xt_hbm.at[0, :, o:o + sz], xbuf.at[0, :, o:o + sz], sems.at[SEM_RAMP + k])
        for k, (o, sz) in enumerate(zip(offs, RAMP))
    ]
    x1_cp = pltpu.make_async_copy(xt_hbm.at[1], xbuf.at[1], sems.at[SEM_X1])
    x23_cp = pltpu.make_async_copy(xt_hbm.at[2:4], xbuf.at[2:4], sems.at[SEM_X23])
    for cp in w_cps + [b_cp] + ramp_cps + [x1_cp, x23_cp]:
        cp.start()
    start_reads(4, 4)

    def prune_scaled(t):
        d, dinv = _pow2(_prune_rows(w_vmem, pk_ref, at_ref, t))
        drow_ref[t:t + 1, :] = d
        return d, dinv

    def make_dcol(t):
        dm = jnp.broadcast_to(drow_ref[t:t + 1, :], (128, 128)).astype(BF16)
        dcol_ref[128 * t:128 * (t + 1), :] = dm.T.astype(F32)

    w_cps[0].wait()
    scale = [prune_scaled(0), prune_scaled(1)]
    w_cps[1].wait()
    make_dcol(0)
    make_dcol(1)
    scale += [prune_scaled(2), prune_scaled(3)]
    w_cps[2].wait()
    make_dcol(2)
    make_dcol(3)
    _prune_rows(w_vmem, pk_ref, at_ref, 4)
    low = lax.broadcasted_iota(jnp.int32, (RC, 128), 1) < 64
    for r in range(0, H, RC):
        a = {}
        for t in range(5):
            for i in range(2):
                v = at_ref[t, i * H + r:i * H + r + RC, :].astype(F32)
                a[i, t] = v * scale[t][1] if t < 4 else v

        def slot_value(pair, ac, xc, half):
            ks = PAIRS[pair]
            m = max(abs(t) for t in ac)
            v = None
            for j, t in enumerate(ac):
                if t != 0:
                    s = a[j // 2, ks[j % 2] // 2]
                    if abs(t) != m:
                        s = s * float(abs(t) / m)
                    v = (s if t > 0 else -s) if v is None else (v + s if t > 0 else v - s)
            if _is_plain(xc) and pair < 4:
                v = v * (scale[ks[xc.index(1) // 2] // 2][0] * float(m))
            elif m != 1:
                v = v * float(m)
            return v if ks[0] % 2 == half else pltpu.roll(v, 64, 1)

        for i, (s0, s1, _) in enumerate(PASSES):
            l_ref[i, r:r + RC, :] = jnp.where(low, slot_value(*s0, 0), slot_value(*s1, 1)).astype(BF16)
    b_cp.wait()
    ramp_cps[0].wait()
    brow = jnp.broadcast_to(b_vmem[...].astype(F32).reshape(1, D), (128, D))
    bcol_ref[...] = brow.astype(BF16).T.astype(F32)

    for k, (o, sz) in enumerate(zip(offs, RAMP)):
        if k > 0:
            ramp_cps[k].wait()
        for c in range(o, o + sz, BW):
            block(0, c)

    HP = NP // 2

    def body(g, carry):
        r = g & 3
        buf = g & 7
        wbuf = buf ^ 4
        last = g == B - 1
        write0 = r == 0
        write1 = jnp.logical_and(r == 1, g > 4)
        read = jnp.logical_and(r == 2, jnp.logical_and(g > 4, g + 2 < B))
        drain = jnp.logical_and(g > B - 4, jnp.logical_not(last))

        pl.when(g == 1)(lambda: x1_cp.wait())
        pl.when(g == 2)(lambda: x23_cp.wait())
        pl.when(write0)(lambda: wait_all(SEM_RMAIN, rows=4 * D - RTAIL))
        pl.when(write1)(lambda: wait_all(SEM_RTAIL, rows=RTAIL))
        pl.when(read)(lambda: wait_all(SEM_WMAIN, tiles=4 * NP - WTAIL))
        pl.when(jnp.logical_and(write0, g >= 8))(lambda: wait_all(SEM_WTAIL, tiles=WTAIL))

        pl.when(jnp.logical_and(read, g > 6))(lambda: start_reads(g + 2, (g + 2) & 7))
        pl.when(jnp.logical_and(write0, g > 8))(lambda: write(g - 4, wbuf, 0, PRE, SEM_WMAIN))
        pl.when(write0)(lambda: write(g - 4, wbuf, PRE, HP, SEM_WMAIN))
        pl.when(last)(lambda: write(g - 1, buf - 1, 0, HP, SEM_LAST))

        def half(b, bbuf, h, sem=SEM_WMAIN, tail_sem=None):
            return functools.partial(write, b, bbuf, h * HP, (h + 1) * HP, sem, tail_sem)

        after = {
            0: [(write0, half(g - 4, wbuf, 1)), (last, half(g - 1, buf - 1, 1, SEM_LAST))],
            1: [(write0, half(g - 3, wbuf + 1, 0)), (write1, half(g - 2, wbuf + 2, 0))],
            2: [(write0, half(g - 3, wbuf + 1, 1)), (write1, half(g - 2, wbuf + 2, 1, tail_sem=SEM_WTAIL))],
            4: [(drain, half(g - 1, buf - 1, 0, SEM_LAST))],
            5: [(drain, half(g - 1, buf - 1, 1, SEM_LAST))],
            9: [(write0, half(g - 2, wbuf + 2, 0))],
            10: [(write0, half(g - 2, wbuf + 2, 1))],
            12: [(g == 3, lambda: write(0, 0, 0, PRE, SEM_WMAIN))],
            13: [(g == 5, lambda: start_reads(8, 0))],
            14: [(g == 7, lambda: write(4, 4, 0, PRE, SEM_WMAIN))],
        }
        ppb = BW // OSUB
        for j in range(S // BW):
            block(buf, j * BW)
            for cond, fn in after.get(j, []):
                pl.when(cond)(fn)
            if j >= 1:
                pl.when(last)(functools.partial(write, g, buf, 0 if j == 1 else j * ppb, (j + 1) * ppb,
                                                SEM_LAST, in_order=True))
        return carry

    lax.fori_loop(1, B, body, 0)
    wait_all(SEM_WMAIN, tiles=4 * NP - WTAIL)
    wait_all(SEM_WTAIL, tiles=WTAIL)
    wait_all(SEM_LAST, tiles=4 * NP)


@jax.jit
def pallas_standalone__structured_sparse_n_m__ragged_kernel(
    x: jax.Array,
    w: jax.Array,
    b: jax.Array,
):
    B, S, D = x.shape
    assert D == 576 and S == sum(RAMP) and BW == 256 and B % 4 == 0 and B >= 12
    _check_scheme()
    nt = pl.cdiv(D, 128)
    out_t = pl.pallas_call(
        _kernel,
        in_specs=[pl.BlockSpec(memory_space=pl.ANY)] * 3,
        out_specs=pl.BlockSpec(memory_space=pl.ANY),
        out_shape=jax.ShapeDtypeStruct((B, D, S), x.dtype),
        scratch_shapes=[
            pltpu.VMEM((8, D, S), BF16),
            pltpu.VMEM((8, D, S), BF16),
            pltpu.VMEM((D, D), BF16),
            pltpu.VMEM((D,), BF16),
            pltpu.VMEM((nt * nt, 64, 128), jnp.int32),
            pltpu.VMEM((nt, D, 128), BF16),
            pltpu.VMEM((8, 128), F32),
            pltpu.VMEM((512, 128), F32),
            pltpu.VMEM((len(PASSES), D // 2, 128), BF16),
            pltpu.VMEM((D, 128), F32),
            pltpu.SemaphoreType.DMA((11 + len(RAMP),)),
        ],
        compiler_params=pltpu.CompilerParams(
            vmem_limit_bytes=96 * 1024 * 1024,
            disable_bounds_checks=True,
            disable_semaphore_checks=True,
        ),
    )(jnp.swapaxes(x, 1, 2), w, b)
    return jnp.swapaxes(out_t, 1, 2)
```

```python
import functools
from fractions import Fraction

import jax
import jax.numpy as jnp
from jax import lax
import jax.experimental.pallas as pl
import jax.experimental.pallas.tpu as pltpu

F32 = jnp.float32
BF16 = jnp.bfloat16

PAIRS = ((0, 2), (1, 3), (4, 6), (5, 7), (8, None))
_H, _Q, _T = Fraction(1, 2), Fraction(1, 4), Fraction(1, 3)
PASSES = (
    ((0, (1, 0, 0, 1), (1, 0, -1, -1)), (4, (_T, 0, _T, 0), (1, -1, 0, 0)), (1, -1, 0, -1)),
    ((0, (0, 0, 1, 1), (1, 0, 0, 0)), (3, (0, 1, 0, 1), (0, 0, 1, -1)), (0, 0, 1, 0)),
    ((0, (1, 0, 0, 0), (1, 1, -1, -1)), (2, (-_H, 0, -_H, 0), (1, -1, 0, 0)), (0, 1, 0, 1)),
    ((0, (0, 0, 0, -1), (1, 0, -1, 0)), (3, (_Q, 0, _Q, 0), (1, -1, 0, 0)), (1, -1, 1, -1)),
    ((0, (1, 1, 0, 0), (0, 0, 1, 1)), (2, (0, 1, 0, 1), (0, 0, 1, -1)), (1, 0, 0, 0)),
    ((0, (-1, 0, 1, 0), (0, 1, 0, 0)), (1, (-1, 0, -1, 0), (1, -1, 0, 0)), (0, 0, 0, 1)),
    ((0, (0, -1, 0, 1), (0, 0, 0, 1)), (1, (0, _H, 0, _H), (0, 0, 1, -1)), (1, -1, 0, 0)),
    ((4, (-_T, 0, _T, 0), (0, 1, 0, 0)), (1, (_H, 0, 0, -_H), (2, 0, -1, -1)), (1, -1, 0, 2)),
    ((1, (0, 0, 1, 1), (1, 0, 0, 0)), (3, (-1, -1, 1, 1), (0, 0, 0, 1)), (0, 0, 1, 1)),
    ((2, (_H, 0, -_H, 0), (0, 1, 0, -1)), (1, (1, 0, 0, 0), (1, 1, -1, -1)), (0, 1, 0, -1)),
    ((1, (0, 0, 0, 1), (1, 0, -1, 0)), (3, (-_H, 0, _H, 0), (0, 1, 0, -1)), (1, -1, -1, 1)),
    ((2, (1, 1, -1, -1), (0, 0, 0, 1)), (1, (_H, _H, 0, 0), (0, 0, 1, 1)), (1, 1, 0, 0)),
    ((2, (_H, 0, -_H, -1), (1, 0, 0, -1)), (4, (_T, 0, 0, 0), (1, 1, 0, 0)), (2, 1, 0, 1)),
    ((2, (0, 0, 1, 1), (1, 0, 0, 0)), (3, (_H, _H, 0, 0), (1, 1, 0, 0)), (1, 1, 1, 1)),
    ((2, (0, 0, 0, 1), (1, 0, -1, 0)), (3, (0, -1, 0, 0), (1, 1, -1, -1)), (1, 0, -1, 0)),
    ((4, (0, 0, -_T, 0), (1, 0, 0, 0)), (3, (_Q, _H, -_Q, 0), (1, 1, 0, -2)), (1, -1, -3, -1)),
)


def _check_scheme():
    for pair, (_, kb) in enumerate(PAIRS):
        members = 1 if kb is None else 2
        for ia in range(4):
            for ix in range(4):
                for ic in range(4):
                    got = sum(ac[ia] * xc[ix] * out[ic]
                              for *slots, out in PASSES for p, ac, xc in slots if p == pair)
                    want = (ia % 2 == ix // 2 < members and ic == 2 * (ia // 2) + ix % 2)
                    assert got == int(want)


_X_RECIPE = {
    (1, 1, 0, 0): ((1, 0, 0, 0), 1, (0, 1, 0, 0)),
    (1, -1, 0, 0): ((1, 0, 0, 0), -1, (0, 1, 0, 0)),
    (0, 0, 1, 1): ((0, 0, 1, 0), 1, (0, 0, 0, 1)),
    (0, 0, 1, -1): ((0, 0, 1, 0), -1, (0, 0, 0, 1)),
    (1, 0, -1, 0): ((1, 0, 0, 0), -1, (0, 0, 1, 0)),
    (0, 1, 0, -1): ((0, 1, 0, 0), -1, (0, 0, 0, 1)),
    (1, 0, 0, -1): ((1, 0, 0, 0), -1, (0, 0, 0, 1)),
    (1, 0, -1, -1): ((1, 0, 0, 0), -1, (0, 0, 1, 1)),
    (1, 1, -1, -1): ((1, 1, 0, 0), -1, (0, 0, 1, 1)),
    (2, 0, -1, -1): ((1, 1, -1, -1), 1, (1, -1, 0, 0)),
    (1, 1, 0, -2): ((1, 0, 0, -1), 1, (0, 1, 0, -1)),
}
_X_RECIPE_PAIR3 = {**_X_RECIPE, (1, 1, -1, -1): ((1, 1, 0, -2), -1, (0, 0, 1, -1))}

RAMP = (256, 512, 1024, 2304)
BW = 256
OSUB = 128
NB = 12
WRITE_START = 12
RC = 16


def _dot(a, b):
    return jnp.dot(a, b, preferred_element_type=F32)


def _mxu_transpose(v):
    r = lax.broadcasted_iota(jnp.int32, (128, 128), 0)
    c = lax.broadcasted_iota(jnp.int32, (128, 128), 1)
    eye = (r == c).astype(BF16)
    return lax.dot_general(eye, v, (((1,), (1,)), ((), ())), preferred_element_type=F32)


def _prune_rows(w_ref, pk_ref, at_ref, t):
    D = w_ref.shape[0]
    r0 = 128 * t
    nr = min(128, D - r0)
    G = nr // 4
    nc = pl.cdiv(D, 128)
    as_f32 = lambda v: lax.bitcast_convert_type(v, F32)
    mag, lo16, hi16 = 0x7FFF0000, 0x0000FFFF, -0x10000
    mx = None
    for c in range(nc):
        lo = c * 128
        wd = min(128, D - lo)
        u = pltpu.bitcast(w_ref[r0:r0 + nr, lo:lo + wd], jnp.int32)
        if wd < 128:
            u = jnp.concatenate([u, jnp.zeros((nr // 2, 128 - wd), jnp.int32)], axis=1)
        pk = pk_ref.at[t * nc + c]
        pk[0:nr // 2, :] = u
        a = pk[pl.ds(0, G, stride=2), :]
        b = pk[pl.ds(1, G, stride=2), :]
        e0 = as_f32((a << 16) & mag)
        e1 = as_f32(a & mag)
        e2 = as_f32((b << 16) & mag)
        e3 = as_f32(b & mag)
        thr = jnp.maximum(jnp.minimum(jnp.maximum(e0, e1), jnp.maximum(e2, e3)),
                          jnp.maximum(jnp.minimum(e0, e1), jnp.minimum(e2, e3)))
        pk[pl.ds(0, G, stride=2), :] = a & (jnp.where(e0 < thr, 0, lo16) | jnp.where(e1 < thr, 0, hi16))
        pk[pl.ds(1, G, stride=2), :] = b & (jnp.where(e2 < thr, 0, lo16) | jnp.where(e3 < thr, 0, hi16))
        u = pk[0:nr // 2, :]
        if nr < 128:
            u = jnp.concatenate([u, jnp.zeros((64 - nr // 2, 128), jnp.int32)], axis=0)
        p = pltpu.bitcast(u, BF16)
        if c < 2 and nr == 128:
            pf = _mxu_transpose(p)
            pt = pf.astype(BF16)
        else:
            pt = p.T
            pf = pt.astype(F32)
        at_ref[t, lo:lo + wd, :] = pt[:wd, :]
        m = jnp.max(jnp.abs(pf[:wd, :]).reshape(wd // 8, 8, 128), axis=0)
        mx = m if mx is None else jnp.maximum(mx, m)
    return jnp.max(mx, axis=0, keepdims=True)


def _pow2(m):
    e = jnp.minimum(lax.bitcast_convert_type(m, jnp.int32) & 0x7F800000, 253 << 23)
    return lax.bitcast_convert_type(e, F32), lax.bitcast_convert_type((254 << 23) - e, F32)


def _is_plain(xc):
    return sum(abs(t) for t in xc) == 1


def _kernel(xt_hbm, w_hbm, b_hbm, o_hbm,
            xbuf, obuf, w_vmem, b_vmem, pk_ref, at_ref, drow_ref, dcol_ref, l_ref, bcol_ref, sems):
    B, D, S = xt_hbm.shape
    H = D // 2
    NP = S // OSUB
    SEM_W, SEM_B = 0, 3
    SEM_X = 4
    SEM_FIRST, SEM_REST = 8, 9
    SEM_RAMP = 10
    HB = B // 2

    def read(g0, g1, sem):
        return pltpu.make_async_copy(xt_hbm.at[g0:g1], xbuf.at[g0 % NB:g0 % NB + g1 - g0], sems.at[sem])

    def write(g, p0, p1, in_order=False):
        buf = jnp.where(g >= NB, g - NB, g)
        sem = jnp.where(g < B - NB, SEM_FIRST, SEM_REST)
        for p in range(p0, p1):
            c = (p if in_order else ((2 * p if 2 * p < NP else 2 * p - NP + 1) + 2) % NP) * OSUB
            pltpu.make_async_copy(obuf.at[buf, :, c:c + OSUB], o_hbm.at[g, :, c:c + OSUB], sems.at[sem]).start()

    def wait_batches(n, sem):
        v = obuf.at[0:n]
        pltpu.make_async_copy(v, v, sems.at[sem]).wait()

    def block(buf, c0):
        x, o = xbuf.at[buf], obuf.at[buf]
        cols = (c0, c0 + BW // 2)
        raw = lambda k, l: x[64 * k:64 * (k + 1), cols[l]:cols[l] + BW // 2]
        cache = {}

        def comb(pair, xc):
            if (pair, xc) not in cache:
                if _is_plain(xc):
                    i = xc.index(1)
                    k = PAIRS[pair][i // 2]
                    v = raw(k, i % 2).astype(F32)
                    if pair < 4:
                        v = v * dcol_ref[64 * k:64 * (k + 1), :]
                else:
                    u, sign, w = (_X_RECIPE_PAIR3 if pair == 3 else _X_RECIPE)[xc]
                    v = comb(pair, u) + comb(pair, w) if sign > 0 else comb(pair, u) - comb(pair, w)
                cache[pair, xc] = v
            return cache[pair, xc]

        def operand(pair, xc):
            if _is_plain(xc):
                i = xc.index(1)
                return raw(PAIRS[pair][i // 2], i % 2)
            return comb(pair, xc).astype(BF16)

        def mm(i):
            return _dot(l_ref[i], jnp.concatenate([operand(p, xc) for p, _, xc in PASSES[i][:2]], axis=0))

        def store(i, l, v):
            o[i * H:(i + 1) * H, cols[l]:cols[l] + BW // 2] = v.astype(BF16)

        bias1, bias2 = bcol_ref[0:H, :], bcol_ref[H:D, :]
        p0, p3, p10, p15 = mm(0), mm(3), mm(10), mm(15)
        v = p3 - p10
        e = p0 + p15
        g = e + (p3 + p10)
        c21 = bias2 + v - 3.0 * p15
        c22 = bias2 - v - e
        p6, p7, p2, p9 = mm(6), mm(7), mm(2), mm(9)
        g = g + p6 + p7
        c11 = bias1 + g
        c12 = bias1 - g + p2 + p9
        c22 = c22 + 2.0 * p7 + p2 - p9
        p11, p12, p13, p8 = mm(11), mm(12), mm(13), mm(8)
        h = p11 + p12 + p13
        u = p8 + p13
        c11 = c11 + h + p12
        store(0, 1, c12 + h)
        c21 = c21 + u
        c22 = c22 + u + p12
        p1, p4, p5, p14 = mm(1), mm(4), mm(5), mm(14)
        store(0, 0, c11 + p4 + p14)
        store(1, 0, c21 + p1 - p14)
        store(1, 1, c22 + p5)

    w_cps = [pltpu.make_async_copy(w_hbm.at[a:b], w_vmem.at[a:b], sems.at[SEM_W + i])
             for i, (a, b) in enumerate([(0, 256), (256, 512), (512, D)])]
    b_cp = pltpu.make_async_copy(b_hbm, b_vmem, sems.at[SEM_B])
    offs = [sum(RAMP[:i]) for i in range(len(RAMP))]
    ramp_cps = [
        pltpu.make_async_copy(xt_hbm.at[0, :, o:o + sz], xbuf.at[0, :, o:o + sz], sems.at[SEM_RAMP + k])
        for k, (o, sz) in enumerate(zip(offs, RAMP))
    ]
    reads = [read(1, 2, SEM_X), read(2, 4, SEM_X + 1), read(4, 8, SEM_X + 2), read(8, NB, SEM_X + 3)]
    for cp in w_cps + [b_cp] + ramp_cps + reads:
        cp.start()

    def prune_scaled(t):
        d, dinv = _pow2(_prune_rows(w_vmem, pk_ref, at_ref, t))
        drow_ref[t:t + 1, :] = d
        return d, dinv

    def make_dcol(t):
        dm = jnp.broadcast_to(drow_ref[t:t + 1, :], (128, 128)).astype(BF16)
        dcol_ref[128 * t:128 * (t + 1), :] = dm.T.astype(F32)

    w_cps[0].wait()
    scale = [prune_scaled(0), prune_scaled(1)]
    w_cps[1].wait()
    make_dcol(0)
    make_dcol(1)
    scale += [prune_scaled(2), prune_scaled(3)]
    w_cps[2].wait()
    make_dcol(2)
    make_dcol(3)
    _prune_rows(w_vmem, pk_ref, at_ref, 4)
    low = lax.broadcasted_iota(jnp.int32, (RC, 128), 1) < 64
    for r in range(0, H, RC):
        a = {}
        for t in range(5):
            for i in range(2):
                v = at_ref[t, i * H + r:i * H + r + RC, :].astype(F32)
                a[i, t] = v * scale[t][1] if t < 4 else v

        def slot_value(pair, ac, xc, half):
            ks = PAIRS[pair]
            m = max(abs(t) for t in ac)
            v = None
            for j, t in enumerate(ac):
                if t != 0:
                    s = a[j // 2, ks[j % 2] // 2]
                    if abs(t) != m:
                        s = s * float(abs(t) / m)
                    v = (s if t > 0 else -s) if v is None else (v + s if t > 0 else v - s)
            if _is_plain(xc) and pair < 4:
                v = v * (scale[ks[xc.index(1) // 2] // 2][0] * float(m))
            elif m != 1:
                v = v * float(m)
            return v if ks[0] % 2 == half else pltpu.roll(v, 64, 1)

        for i, (s0, s1, _) in enumerate(PASSES):
            l_ref[i, r:r + RC, :] = jnp.where(low, slot_value(*s0, 0), slot_value(*s1, 1)).astype(BF16)
    b_cp.wait()
    ramp_cps[0].wait()
    brow = jnp.broadcast_to(b_vmem[...].astype(F32).reshape(1, D), (128, D))
    bcol_ref[...] = brow.astype(BF16).T.astype(F32)

    for k, (o, sz) in enumerate(zip(offs, RAMP)):
        if k > 0:
            ramp_cps[k].wait()
        for c in range(o, o + sz, BW):
            block(0, c)

    HP = NP // 2

    def body(g, carry):
        buf = jnp.where(g >= NB, g - NB, g)
        last = g == B - 1
        writing = g >= HB
        wb = jnp.minimum(2 * (g - HB) + 1, g - 1)
        two = jnp.logical_and(writing, g < B - 2)

        for k in range(4):
            pl.when(g == 1 << k)(functools.partial(wait_batches, 1 << k, SEM_X + k))
        pl.when(g == NB)(lambda: wait_batches(B - NB, SEM_FIRST))
        pl.when(g == B - NB)(lambda: read(NB, B, SEM_X + 3).start())

        pl.when(writing)(lambda: write(wb, 0, HP))
        after = {
            1: (writing, lambda: write(wb, HP, NP)),
            6: (two, lambda: write(wb + 1, 0, HP)),
            11: (two, lambda: write(wb + 1, HP, NP)),
            WRITE_START: (g == HB - 1, lambda: write(0, 0, HP)),
            WRITE_START + 1: (g == HB - 1, lambda: write(0, HP, NP)),
        }
        ppb = BW // OSUB
        for j in range(S // BW):
            block(buf, j * BW)
            if j in after:
                pl.when(after[j][0])(after[j][1])
            if j >= 2:
                pl.when(last)(functools.partial(write, g, 0 if j == 2 else j * ppb, (j + 1) * ppb,
                                                in_order=True))
        return carry

    lax.fori_loop(1, B, body, 0)
    wait_batches(NB, SEM_REST)


@jax.jit
def pallas_standalone__structured_sparse_n_m__ragged_kernel(
    x: jax.Array,
    w: jax.Array,
    b: jax.Array,
):
    B, S, D = x.shape
    assert D == 576 and S == sum(RAMP) and BW == 256 and B == 16
    _check_scheme()
    nt = pl.cdiv(D, 128)
    out_t = pl.pallas_call(
        _kernel,
        in_specs=[pl.BlockSpec(memory_space=pl.ANY)] * 3,
        out_specs=pl.BlockSpec(memory_space=pl.ANY),
        out_shape=jax.ShapeDtypeStruct((B, D, S), x.dtype),
        scratch_shapes=[
            pltpu.VMEM((NB, D, S), BF16),
            pltpu.VMEM((NB, D, S), BF16),
            pltpu.VMEM((D, D), BF16),
            pltpu.VMEM((D,), BF16),
            pltpu.VMEM((nt * nt, 64, 128), jnp.int32),
            pltpu.VMEM((nt, D, 128), BF16),
            pltpu.VMEM((8, 128), F32),
            pltpu.VMEM((512, 128), F32),
            pltpu.VMEM((len(PASSES), D // 2, 128), BF16),
            pltpu.VMEM((D, 128), F32),
            pltpu.SemaphoreType.DMA((10 + len(RAMP),)),
        ],
        compiler_params=pltpu.CompilerParams(
            vmem_limit_bytes=116 * 1024 * 1024,
            disable_bounds_checks=True,
            disable_semaphore_checks=True,
        ),
    )(jnp.swapaxes(x, 1, 2), w, b)
    return jnp.swapaxes(out_t, 1, 2)
```

```python
import functools
from fractions import Fraction

import jax
import jax.numpy as jnp
from jax import lax
import jax.experimental.pallas as pl
import jax.experimental.pallas.tpu as pltpu

F32 = jnp.float32
BF16 = jnp.bfloat16

PAIRS = ((0, 2), (1, 3), (4, 6), (5, 7), (8, None))
_H, _Q, _T = Fraction(1, 2), Fraction(1, 4), Fraction(1, 3)
PASSES = (
    ((0, (1, 0, 0, 1), (1, 0, -1, -1)), (4, (_T, 0, _T, 0), (1, -1, 0, 0)), (1, -1, 0, -1)),
    ((0, (0, 0, 1, 1), (1, 0, 0, 0)), (3, (0, 1, 0, 1), (0, 0, 1, -1)), (0, 0, 1, 0)),
    ((0, (1, 0, 0, 0), (1, 1, -1, -1)), (2, (-_H, 0, -_H, 0), (1, -1, 0, 0)), (0, 1, 0, 1)),
    ((0, (0, 0, 0, -1), (1, 0, -1, 0)), (3, (_Q, 0, _Q, 0), (1, -1, 0, 0)), (1, -1, 1, -1)),
    ((0, (1, 1, 0, 0), (0, 0, 1, 1)), (2, (0, 1, 0, 1), (0, 0, 1, -1)), (1, 0, 0, 0)),
    ((0, (-1, 0, 1, 0), (0, 1, 0, 0)), (1, (-1, 0, -1, 0), (1, -1, 0, 0)), (0, 0, 0, 1)),
    ((0, (0, -1, 0, 1), (0, 0, 0, 1)), (1, (0, _H, 0, _H), (0, 0, 1, -1)), (1, -1, 0, 0)),
    ((4, (-_T, 0, _T, 0), (0, 1, 0, 0)), (1, (_H, 0, 0, -_H), (2, 0, -1, -1)), (1, -1, 0, 2)),
    ((1, (0, 0, 1, 1), (1, 0, 0, 0)), (3, (-1, -1, 1, 1), (0, 0, 0, 1)), (0, 0, 1, 1)),
    ((2, (_H, 0, -_H, 0), (0, 1, 0, -1)), (1, (1, 0, 0, 0), (1, 1, -1, -1)), (0, 1, 0, -1)),
    ((1, (0, 0, 0, 1), (1, 0, -1, 0)), (3, (-_H, 0, _H, 0), (0, 1, 0, -1)), (1, -1, -1, 1)),
    ((2, (1, 1, -1, -1), (0, 0, 0, 1)), (1, (_H, _H, 0, 0), (0, 0, 1, 1)), (1, 1, 0, 0)),
    ((2, (_H, 0, -_H, -1), (1, 0, 0, -1)), (4, (_T, 0, 0, 0), (1, 1, 0, 0)), (2, 1, 0, 1)),
    ((2, (0, 0, 1, 1), (1, 0, 0, 0)), (3, (_H, _H, 0, 0), (1, 1, 0, 0)), (1, 1, 1, 1)),
    ((2, (0, 0, 0, 1), (1, 0, -1, 0)), (3, (0, -1, 0, 0), (1, 1, -1, -1)), (1, 0, -1, 0)),
    ((4, (0, 0, -_T, 0), (1, 0, 0, 0)), (3, (_Q, _H, -_Q, 0), (1, 1, 0, -2)), (1, -1, -3, -1)),
)


def _check_scheme():
    for pair, (_, kb) in enumerate(PAIRS):
        members = 1 if kb is None else 2
        for ia in range(4):
            for ix in range(4):
                for ic in range(4):
                    got = sum(ac[ia] * xc[ix] * out[ic]
                              for *slots, out in PASSES for p, ac, xc in slots if p == pair)
                    want = (ia % 2 == ix // 2 < members and ic == 2 * (ia // 2) + ix % 2)
                    assert got == int(want)


_X_RECIPE = {
    (1, 1, 0, 0): ((1, 0, 0, 0), 1, (0, 1, 0, 0)),
    (1, -1, 0, 0): ((1, 0, 0, 0), -1, (0, 1, 0, 0)),
    (0, 0, 1, 1): ((0, 0, 1, 0), 1, (0, 0, 0, 1)),
    (0, 0, 1, -1): ((0, 0, 1, 0), -1, (0, 0, 0, 1)),
    (1, 0, -1, 0): ((1, 0, 0, 0), -1, (0, 0, 1, 0)),
    (0, 1, 0, -1): ((0, 1, 0, 0), -1, (0, 0, 0, 1)),
    (1, 0, 0, -1): ((1, 0, 0, 0), -1, (0, 0, 0, 1)),
    (1, 0, -1, -1): ((1, 0, 0, 0), -1, (0, 0, 1, 1)),
    (1, 1, -1, -1): ((1, 1, 0, 0), -1, (0, 0, 1, 1)),
    (2, 0, -1, -1): ((1, 1, -1, -1), 1, (1, -1, 0, 0)),
    (1, 1, 0, -2): ((1, 0, 0, -1), 1, (0, 1, 0, -1)),
}
_X_RECIPE_PAIR3 = {**_X_RECIPE, (1, 1, -1, -1): ((1, 1, 0, -2), -1, (0, 0, 1, -1))}

RAMP = (256, 512, 1024, 2304)
BW = 256
OSUB = 128
NB = 12
WRITE_START = 12
RC = 16


def _dot(a, b):
    return jnp.dot(a, b, preferred_element_type=F32)


def _mxu_transpose(v):
    r = lax.broadcasted_iota(jnp.int32, (128, 128), 0)
    c = lax.broadcasted_iota(jnp.int32, (128, 128), 1)
    eye = (r == c).astype(BF16)
    return lax.dot_general(eye, v, (((1,), (1,)), ((), ())), preferred_element_type=F32)


def _prune_rows(w_ref, pk_ref, at_ref, t):
    D = w_ref.shape[0]
    r0 = 128 * t
    nr = min(128, D - r0)
    G = nr // 4
    nc = pl.cdiv(D, 128)
    as_f32 = lambda v: lax.bitcast_convert_type(v, F32)
    mag, lo16, hi16 = 0x7FFF0000, 0x0000FFFF, -0x10000
    mx = None
    for c in range(nc):
        lo = c * 128
        wd = min(128, D - lo)
        u = pltpu.bitcast(w_ref[r0:r0 + nr, lo:lo + wd], jnp.int32)
        if wd < 128:
            u = jnp.concatenate([u, jnp.zeros((nr // 2, 128 - wd), jnp.int32)], axis=1)
        pk = pk_ref.at[t * nc + c]
        pk[0:nr // 2, :] = u
        a = pk[pl.ds(0, G, stride=2), :]
        b = pk[pl.ds(1, G, stride=2), :]
        e0 = as_f32((a << 16) & mag)
        e1 = as_f32(a & mag)
        e2 = as_f32((b << 16) & mag)
        e3 = as_f32(b & mag)
        thr = jnp.maximum(jnp.minimum(jnp.maximum(e0, e1), jnp.maximum(e2, e3)),
                          jnp.maximum(jnp.minimum(e0, e1), jnp.minimum(e2, e3)))
        pk[pl.ds(0, G, stride=2), :] = a & (jnp.where(e0 < thr, 0, lo16) | jnp.where(e1 < thr, 0, hi16))
        pk[pl.ds(1, G, stride=2), :] = b & (jnp.where(e2 < thr, 0, lo16) | jnp.where(e3 < thr, 0, hi16))
        u = pk[0:nr // 2, :]
        if nr < 128:
            u = jnp.concatenate([u, jnp.zeros((64 - nr // 2, 128), jnp.int32)], axis=0)
        p = pltpu.bitcast(u, BF16)
        if c < 2 and nr == 128:
            pf = _mxu_transpose(p)
            pt = pf.astype(BF16)
        else:
            pt = p.T
            pf = pt.astype(F32)
        at_ref[t, lo:lo + wd, :] = pt[:wd, :]
        m = jnp.max(jnp.abs(pf[:wd, :]).reshape(wd // 8, 8, 128), axis=0)
        mx = m if mx is None else jnp.maximum(mx, m)
    return jnp.max(mx, axis=0, keepdims=True)


def _pow2(m):
    e = jnp.minimum(lax.bitcast_convert_type(m, jnp.int32) & 0x7F800000, 253 << 23)
    return lax.bitcast_convert_type(e, F32), lax.bitcast_convert_type((254 << 23) - e, F32)


def _is_plain(xc):
    return sum(abs(t) for t in xc) == 1


def _kernel(xt_hbm, w_hbm, b_hbm, o_hbm,
            xbuf, obuf, w_vmem, b_vmem, pk_ref, at_ref, drow_ref, dcol_ref, l_ref, bcol_ref, sems):
    B, D, S = xt_hbm.shape
    H = D // 2
    NP = S // OSUB
    SEM_W, SEM_B = 0, 3
    SEM_X = 4
    SEM_FIRST, SEM_REST = 9, 10
    SEM_RAMP = 11
    HB = B // 2

    def read(g0, g1, sem):
        return pltpu.make_async_copy(xt_hbm.at[g0:g1], xbuf.at[g0 % NB:g0 % NB + g1 - g0], sems.at[sem])

    def write(g, p0, p1, in_order=False):
        buf = jnp.where(g >= NB, g - NB, g)
        sem = jnp.where(g < B - NB, SEM_FIRST, SEM_REST)
        for p in range(p0, p1):
            c = (p if in_order else ((2 * p if 2 * p < NP else 2 * p - NP + 1) + 2) % NP) * OSUB
            pltpu.make_async_copy(obuf.at[buf, :, c:c + OSUB], o_hbm.at[g, :, c:c + OSUB], sems.at[sem]).start()

    def wait_writes(n, sem):
        v = obuf.at[0:n]
        pltpu.make_async_copy(v, v, sems.at[sem]).wait()

    def block(buf, c0):
        x, o = xbuf.at[buf], obuf.at[buf]
        cols = (c0, c0 + BW // 2)
        raw = lambda k, l: x[64 * k:64 * (k + 1), cols[l]:cols[l] + BW // 2]
        cache = {}

        def comb(pair, xc):
            if (pair, xc) not in cache:
                if _is_plain(xc):
                    i = xc.index(1)
                    k = PAIRS[pair][i // 2]
                    v = raw(k, i % 2).astype(F32)
                    if pair < 4:
                        v = v * dcol_ref[64 * k:64 * (k + 1), :]
                else:
                    u, sign, w = (_X_RECIPE_PAIR3 if pair == 3 else _X_RECIPE)[xc]
                    v = comb(pair, u) + comb(pair, w) if sign > 0 else comb(pair, u) - comb(pair, w)
                cache[pair, xc] = v
            return cache[pair, xc]

        def operand(pair, xc):
            if _is_plain(xc):
                i = xc.index(1)
                return raw(PAIRS[pair][i // 2], i % 2)
            return comb(pair, xc).astype(BF16)

        def mm(i):
            return _dot(l_ref[i], jnp.concatenate([operand(p, xc) for p, _, xc in PASSES[i][:2]], axis=0))

        def store(i, l, v):
            o[i * H:(i + 1) * H, cols[l]:cols[l] + BW // 2] = v.astype(BF16)

        bias1, bias2 = bcol_ref[0:H, :], bcol_ref[H:D, :]
        p0, p3, p10, p15 = mm(0), mm(3), mm(10), mm(15)
        v = p3 - p10
        e = p0 + p15
        g = e + (p3 + p10)
        c21 = bias2 + v - 3.0 * p15
        c22 = bias2 - v - e
        p6, p7, p2, p9 = mm(6), mm(7), mm(2), mm(9)
        g = g + p6 + p7
        c11 = bias1 + g
        c12 = bias1 - g + p2 + p9
        c22 = c22 + 2.0 * p7 + p2 - p9
        p11, p12, p13, p8 = mm(11), mm(12), mm(13), mm(8)
        h = p11 + p12 + p13
        u = p8 + p13
        c11 = c11 + h + p12
        store(0, 1, c12 + h)
        c21 = c21 + u
        c22 = c22 + u + p12
        p1, p4, p5, p14 = mm(1), mm(4), mm(5), mm(14)
        store(0, 0, c11 + p4 + p14)
        store(1, 0, c21 + p1 - p14)
        store(1, 1, c22 + p5)

    w_cps = [pltpu.make_async_copy(w_hbm.at[a:b], w_vmem.at[a:b], sems.at[SEM_W + i])
             for i, (a, b) in enumerate([(0, 256), (256, 512), (512, D)])]
    b_cp = pltpu.make_async_copy(b_hbm, b_vmem, sems.at[SEM_B])
    offs = [sum(RAMP[:i]) for i in range(len(RAMP))]
    ramp_cps = [
        pltpu.make_async_copy(xt_hbm.at[0, :, o:o + sz], xbuf.at[0, :, o:o + sz], sems.at[SEM_RAMP + k])
        for k, (o, sz) in enumerate(zip(offs, RAMP))
    ]
    reads = [read(1, 2, SEM_X), read(2, 4, SEM_X + 1), read(4, 8, SEM_X + 2), read(8, NB, SEM_X + 3)]
    late_read = read(NB, B, SEM_X + 4)
    for cp in w_cps + [b_cp] + ramp_cps + reads:
        cp.start()

    def prune_scaled(t):
        d, dinv = _pow2(_prune_rows(w_vmem, pk_ref, at_ref, t))
        drow_ref[t:t + 1, :] = d
        return d, dinv

    def make_dcol(t):
        dm = jnp.broadcast_to(drow_ref[t:t + 1, :], (128, 128)).astype(BF16)
        dcol_ref[128 * t:128 * (t + 1), :] = dm.T.astype(F32)

    w_cps[0].wait()
    scale = [prune_scaled(0), prune_scaled(1)]
    w_cps[1].wait()
    make_dcol(0)
    make_dcol(1)
    scale += [prune_scaled(2), prune_scaled(3)]
    w_cps[2].wait()
    make_dcol(2)
    make_dcol(3)
    _prune_rows(w_vmem, pk_ref, at_ref, 4)
    low = lax.broadcasted_iota(jnp.int32, (RC, 128), 1) < 64
    for r in range(0, H, RC):
        a = {}
        for t in range(5):
            for i in range(2):
                v = at_ref[t, i * H + r:i * H + r + RC, :].astype(F32)
                a[i, t] = v * scale[t][1] if t < 4 else v

        def slot_value(pair, ac, xc, half):
            ks = PAIRS[pair]
            m = max(abs(t) for t in ac)
            v = None
            for j, t in enumerate(ac):
                if t != 0:
                    s = a[j // 2, ks[j % 2] // 2]
                    if abs(t) != m:
                        s = s * float(abs(t) / m)
                    v = (s if t > 0 else -s) if v is None else (v + s if t > 0 else v - s)
            if _is_plain(xc) and pair < 4:
                v = v * (scale[ks[xc.index(1) // 2] // 2][0] * float(m))
            elif m != 1:
                v = v * float(m)
            return v if ks[0] % 2 == half else pltpu.roll(v, 64, 1)

        for i, (s0, s1, _) in enumerate(PASSES):
            l_ref[i, r:r + RC, :] = jnp.where(low, slot_value(*s0, 0), slot_value(*s1, 1)).astype(BF16)
    b_cp.wait()
    ramp_cps[0].wait()
    brow = jnp.broadcast_to(b_vmem[...].astype(F32).reshape(1, D), (128, D))
    bcol_ref[...] = brow.astype(BF16).T.astype(F32)

    for k, (o, sz) in enumerate(zip(offs, RAMP)):
        if k > 0:
            ramp_cps[k].wait()
        for c in range(o, o + sz, BW):
            block(0, c)

    HP = NP // 2

    def body(g, carry):
        buf = jnp.where(g >= NB, g - NB, g)
        last = g == B - 1
        writing = g >= HB
        wb = jnp.minimum(2 * (g - HB) + 1, g - 1)
        two = jnp.logical_and(writing, g < B - 2)

        for first, cp in zip((1, 2, 4, 8, NB), reads + [late_read]):
            pl.when(g == first)(cp.wait)
        pl.when(g == NB)(lambda: wait_writes(B - NB, SEM_FIRST))
        pl.when(g == B - NB)(late_read.start)

        pl.when(writing)(lambda: write(wb, 0, HP))
        after = {
            1: (writing, lambda: write(wb, HP, NP)),
            6: (two, lambda: write(wb + 1, 0, HP)),
            11: (two, lambda: write(wb + 1, HP, NP)),
            WRITE_START: (g == HB - 1, lambda: write(0, 0, HP)),
            WRITE_START + 1: (g == HB - 1, lambda: write(0, HP, NP)),
        }
        ppb = BW // OSUB
        for j in range(S // BW):
            block(buf, j * BW)
            if j in after:
                pl.when(after[j][0])(after[j][1])
            if j >= 2:
                pl.when(last)(functools.partial(write, g, 0 if j == 2 else j * ppb, (j + 1) * ppb,
                                                in_order=True))
        return carry

    lax.fori_loop(1, B, body, 0)
    wait_writes(NB, SEM_REST)


@jax.jit
def pallas_standalone__structured_sparse_n_m__ragged_kernel(
    x: jax.Array,
    w: jax.Array,
    b: jax.Array,
):
    B, S, D = x.shape
    assert D == 576 and S == sum(RAMP) and BW == 256 and B == 16
    _check_scheme()
    nt = pl.cdiv(D, 128)
    out_t = pl.pallas_call(
        _kernel,
        in_specs=[pl.BlockSpec(memory_space=pl.ANY)] * 3,
        out_specs=pl.BlockSpec(memory_space=pl.ANY),
        out_shape=jax.ShapeDtypeStruct((B, D, S), x.dtype),
        scratch_shapes=[
            pltpu.VMEM((NB, D, S), BF16),
            pltpu.VMEM((NB, D, S), BF16),
            pltpu.VMEM((D, D), BF16),
            pltpu.VMEM((D,), BF16),
            pltpu.VMEM((nt * nt, 64, 128), jnp.int32),
            pltpu.VMEM((nt, D, 128), BF16),
            pltpu.VMEM((8, 128), F32),
            pltpu.VMEM((512, 128), F32),
            pltpu.VMEM((len(PASSES), D // 2, 128), BF16),
            pltpu.VMEM((D, 128), F32),
            pltpu.SemaphoreType.DMA((11 + len(RAMP),)),
        ],
        compiler_params=pltpu.CompilerParams(
            vmem_limit_bytes=116 * 1024 * 1024,
            **{k: True for k in ("disable_bounds_checks", "disable_semaphore_checks")
               if k in pltpu.CompilerParams.__dataclass_fields__},
        ),
    )(jnp.swapaxes(x, 1, 2), w, b)
    return jnp.swapaxes(out_t, 1, 2)
```
